```python
import jax
import jax.numpy as jnp

def _softmax(x, axis=-1):
    return jax.nn.softmax(x, axis=axis)
def _gelu(x):
    return jax.nn.gelu(x, approximate=True)
def _silu(x):
    return jax.nn.silu(x)
def _sigmoid(x):
    return jax.nn.sigmoid(x)
def _layernorm(x, axis=-1, eps=1e-5):
    m = jnp.mean(x, axis=axis, keepdims=True)
    v = jnp.var(x, axis=axis, keepdims=True)
    return (x - m) / jnp.sqrt(v + eps)
def _scatter_add(tgt, idx, src, axis=0):
    return tgt.at[idx].add(src)
def _segment_sum(src, seg, n):
    return jax.ops.segment_sum(src, seg, n)
class _Rng:
    def __init__(self, key):
        self._k = key
    def _next(self):
        self._k, sub = jax.random.split(self._k)
        return sub
    def normal(self, shape):
        return jax.random.normal(self._next(), shape, dtype=jnp.bfloat16)
    def randint(self, lo, hi, shape):
        return jax.random.randint(self._next(), shape, lo, hi, dtype=jnp.int32)
    def uniform(self, shape, lo=0.0, hi=1.0):
        return jax.random.uniform(self._next(), shape, jnp.bfloat16, lo, hi)
    def permutation(self, n):
        return jax.random.permutation(self._next(), n)


kernel_name = 'concat_heads__compressed_kv_cla__sliding_local_dilated__prompt'

def setup_inputs():
    _rng = _Rng(jax.random.key(int.from_bytes(__import__("os").urandom(4), "little")))
    _w = (lambda a: (lambda t: t.astype(jnp.bfloat16) if jnp.issubdtype(t.dtype, jnp.floating) else t)(jnp.asarray(a)))
    def _A_setup():
        B, H, Sq, Sk, D, M = 1, 32, 2048, 2048, 128, 1024
        Dc = 4 * D
        return {
            "x": _w((lambda *s: _rng.normal(s) * 0.05)(B, Sq, M)),
            "c_kv": _w((lambda *s: _rng.normal(s) * 0.05)(B, Sk, Dc)),
            "w_q": _w((lambda *s: _rng.normal(s) * 0.05)(M, H, D) * (M ** -0.5)),
            "w_uk": _w((lambda *s: _rng.normal(s) * 0.05)(Dc, H, D) * (Dc ** -0.5)),
            "w_uv": _w((lambda *s: _rng.normal(s) * 0.05)(Dc, H, D) * (Dc ** -0.5)),
            "w_o": _w((lambda *s: _rng.normal(s) * 0.05)(H, D, M) * ((H * D) ** -0.5)),
        }
    _A_in = _A_setup()

    def _B_setup():
        B, S, D = 1, 2048, 1024
        return {
            "x": _w((lambda *s: _rng.normal(s) * 0.05)(B, S, D)),
            "wqkv": _w((lambda *s: _rng.normal(s) * 0.05)(D, 3 * D)),
            "wo": _w((lambda *s: _rng.normal(s) * 0.05)(D, D)),
        }
    _B_in = _B_setup()

    return {
        "A_x": _A_in["x"],
        "A_c_kv": _A_in["c_kv"],
        "A_w_q": _A_in["w_q"],
        "A_w_uk": _A_in["w_uk"],
        "A_w_uv": _A_in["w_uv"],
        "A_w_o": _A_in["w_o"],
        "B_x": _B_in["x"],
        "B_wqkv": _B_in["wqkv"],
        "B_wo": _B_in["wo"],
    }

def reference(A_x, A_c_kv, A_w_q, A_w_uk, A_w_uv, A_w_o, B_x, B_wqkv, B_wo):
    def _A_ref(x, c_kv, w_q, w_uk, w_uv, w_o):
        B, Sq, M = x.shape[0], x.shape[1], x.shape[2]
        Sk = c_kv.shape[1]
        H, D = w_q.shape[1], w_q.shape[2]
        q = jnp.einsum("bqm,mhd->bhqd", x, w_q)
        k = jnp.einsum("bkc,chd->bhkd", c_kv, w_uk)
        v = jnp.einsum("bkc,chd->bhkd", c_kv, w_uv)
        scores = jnp.einsum("bhqd,bhkd->bhqk", q, k) * (D ** -0.5)
        off = Sk - Sq
        qi = jnp.arange(Sq)[:, None]
        kj = jnp.arange(Sk)[None, :]
        cmask = kj <= (qi + off)
        scores = jnp.where(cmask[None, None], scores, -1e9)
        p = _softmax(scores, axis=-1)
        ctx = jnp.einsum("bhqk,bhkd->bhqd", p, v)
        return jnp.einsum("bhqd,hdm->bqm", ctx, w_o)

    def _B_ref(x, wqkv, wo):
        B, S, D = x.shape
        H = 32; Dh = D // H
        W, dil = 8, 2
        qkv = (lambda x, *d: x.transpose(*d))((x @ wqkv).reshape(B, S, 3, H, Dh), 2, 0, 3, 1, 4)
        q, k, v = qkv[0], qkv[1], qkv[2]
        scale = Dh ** -0.5
        pos = jnp.arange(S)
        off = jnp.arange(W) * dil
        idx = pos[:, None] - off[None, :]
        mask = idx >= 0
        idx_c = jnp.where(mask, idx, 0).reshape(-1)
        kg = k[:, :, idx_c, :].reshape(B, H, S, W, Dh)
        vg = v[:, :, idx_c, :].reshape(B, H, S, W, Dh)
        logits = jnp.einsum("bhsd,bhswd->bhsw", q, kg) * scale
        logits = jnp.where(mask[None, None, :, :], logits, -1e9)
        attn = _softmax(logits, axis=-1)
        o = jnp.einsum("bhsw,bhswd->bhsd", attn, vg)
        return (lambda x, *d: x.transpose(*d))(o, 0, 2, 1, 3).reshape(B, S, D) @ wo

    a = _A_ref(A_x, A_c_kv, A_w_q, A_w_uk, A_w_uv, A_w_o)
    b = _B_ref(B_x, B_wqkv, B_wo)
    return jnp.concatenate([a, b], axis=-1)
```

```python
import jax
import jax.numpy as jnp
import jax.experimental.pallas as pl
import jax.experimental.pallas.tpu as pltpu

bf16 = jnp.bfloat16
f32 = jnp.float32

S = 2048
H = 32
D = 128
M = 1024
DC = 512
HG = 8
NG = H // HG
BQ = 256
NQ = S // BQ
HB = 128
BW = 8
BDIL = 2
BH = 32
BDH = 32
HALO = 16
BR = 256
NB = S // BR
CH = 32
LOG2E = 1.4426950408889634
NEG = -1e30
NT = (((1,), (1,)), ((), ()))


def _dot(a, b):
    return jnp.dot(a, b, preferred_element_type=f32)


def _dot_nt(a, b):
    return jax.lax.dot_general(a, b, NT, preferred_element_type=f32)


def _recip(x):
    return 1.0 / x


def _kernel(x_hbm, c_hbm, wq_hbm, wuk_hbm, wuv_hbm, wo_hbm, xb_hbm, wqkv_hbm, wob_hbm,
            o_ref,
            x_s, c_s, rawq, rawk, rawv, tq, tk, tv,
            wq_cur, wkv_cur, wq_nxt, wkv_nxt,
            qa, ka, va, v0n, ctx_s, wo_s, xb_s, wqkv_s, wob_s,
            wt_s, wobp_s, tb, qb_s, kb_s, vb_s, ob_s, sems):
    step = pl.program_id(0)

    SEM_X, SEM_C, SEM_Q, SEM_K, SEM_V = 0, 1, 2, 6, 10
    SEM_WO, SEM_XB, SEM_WQKV, SEM_WOB = 14, 15, 16, 17

    def cp_x():
        return pltpu.make_async_copy(x_hbm, x_s, sems.at[SEM_X])

    def cp_c():
        return pltpu.make_async_copy(c_hbm, c_s, sems.at[SEM_C])

    def cp_group(g):
        return [
            pltpu.make_async_copy(wq_hbm.at[:, pl.ds(g * HG, HG), :], rawq.at[g], sems.at[SEM_Q + g]),
            pltpu.make_async_copy(wuk_hbm.at[:, pl.ds(g * HG, HG), :], rawk.at[g], sems.at[SEM_K + g]),
            pltpu.make_async_copy(wuv_hbm.at[:, pl.ds(g * HG, HG), :], rawv.at[g], sems.at[SEM_V + g]),
        ]

    def cp_rest():
        return [
            pltpu.make_async_copy(wqkv_hbm, wqkv_s, sems.at[SEM_WQKV]),
            pltpu.make_async_copy(wob_hbm, wob_s, sems.at[SEM_WOB]),
            pltpu.make_async_copy(wo_hbm, wo_s, sems.at[SEM_WO]),
            pltpu.make_async_copy(xb_hbm, xb_s, sems.at[SEM_XB]),
        ]

    def convert_slice(g, par, sl):
        mq = M // HG
        m0 = pl.multiple_of(sl * mq, mq)
        tq[par, pl.ds(m0 * HG, mq * HG), :] = (
            rawq[g, pl.ds(m0, mq)].astype(f32).reshape(mq * HG, D))
        mk = DC // HG
        k0 = pl.multiple_of(sl * mk, mk)
        tk[par, pl.ds(k0 * HG, mk * HG), :] = (
            rawk[g, pl.ds(k0, mk)].astype(f32).reshape(mk * HG, D))
        tv[par, pl.ds(k0 * HG, mk * HG), :] = (
            rawv[g, pl.ds(k0, mk)].astype(f32).reshape(mk * HG, D))

    def extract(par, j):
        wq_nxt[...] = tq[par, pl.ds(j, M, stride=HG), :].astype(bf16)
        wkv_nxt[:, 0:D] = tk[par, pl.ds(j, DC, stride=HG), :].astype(bf16)
        wkv_nxt[:, D:2 * D] = tv[par, pl.ds(j, DC, stride=HG), :].astype(bf16)

    def proj(i, wq, wkv, v_first=False):
        r = slice(i * BQ, (i + 1) * BQ)
        q = _dot(x_s[r, :], wq[...])
        qa[r, :] = (q * (D ** -0.5 * LOG2E)).astype(bf16)
        kv = _dot(c_s[r, :], wkv[...])
        ka[r, :] = kv[:, :D].astype(bf16)
        if v_first:
            v0n[...] = kv[:, D:].astype(bf16)
        else:
            va[r, :] = kv[:, D:].astype(bf16)

    def qk(i):
        r0 = i * BQ
        q = qa[r0:r0 + BQ, :]
        s_main = _dot_nt(q, ka[0:r0 + HB, :])
        s_ext = _dot_nt(q[HB:], ka[r0 + HB:r0 + BQ, :])
        return s_main, s_ext

    def softmax_pv(h, i, s_main, s_ext, tri):
        r0 = i * BQ
        top_d = jnp.where(tri, s_main[:HB, r0:], NEG)
        ext = jnp.where(tri, s_ext, NEG)
        bot = s_main[HB:, :]
        m_top = jnp.max(top_d, axis=1, keepdims=True)
        if i > 0:
            top_o = s_main[:HB, :r0]
            m_top = jnp.maximum(m_top, jnp.max(top_o, axis=1, keepdims=True))
        m_bot = jnp.maximum(jnp.max(bot, axis=1, keepdims=True),
                            jnp.max(ext, axis=1, keepdims=True))
        p_topd = jnp.exp2(top_d - m_top)
        l_top = jnp.sum(p_topd, axis=1, keepdims=True)
        if i > 0:
            p_topo = jnp.exp2(top_o - m_top)
            l_top = l_top + jnp.sum(p_topo, axis=1, keepdims=True)
            p_top = jnp.concatenate([p_topo.astype(bf16), p_topd.astype(bf16)], axis=1)
        else:
            p_top = p_topd.astype(bf16)
        p_bot = jnp.exp2(bot - m_bot)
        p_ext = jnp.exp2(ext - m_bot)
        l_bot = jnp.sum(p_bot, axis=1, keepdims=True) + jnp.sum(p_ext, axis=1, keepdims=True)
        p_main = jnp.concatenate([p_top, p_bot.astype(bf16)], axis=0)
        c_main = _dot(p_main, va[0:r0 + HB, :])
        c_ext = _dot(p_ext.astype(bf16), va[r0 + HB:r0 + BQ, :])
        ctx_s[h, r0:r0 + HB, :] = (c_main[:HB] * _recip(l_top)).astype(bf16)
        ctx_s[h, r0 + HB:r0 + BQ, :] = ((c_main[HB:] + c_ext) * _recip(l_bot)).astype(bf16)

    def head_body(h, carry):
        hn = h + 1

        @pl.when(jnp.logical_and(hn % HG == 0, hn // HG + 1 < NG))
        def _():
            g = hn // HG + 1
            pltpu.make_async_copy(wq_hbm.at[:, pl.ds(0, HG), :], rawq.at[g], sems.at[SEM_Q + g]).wait()
            pltpu.make_async_copy(wuk_hbm.at[:, pl.ds(0, HG), :], rawk.at[g], sems.at[SEM_K + g]).wait()
            pltpu.make_async_copy(wuv_hbm.at[:, pl.ds(0, HG), :], rawv.at[g], sems.at[SEM_V + g]).wait()

        row = jax.lax.broadcasted_iota(jnp.int32, (HB, HB), 0)
        col = jax.lax.broadcasted_iota(jnp.int32, (HB, HB), 1)
        tri = col <= row

        wq_cur[...] = wq_nxt[...]
        wkv_cur[...] = wkv_nxt[...]
        va[0:BQ, :] = v0n[...]
        for i in range(NQ):
            s_main, s_ext = qk(i)
            if i + 1 < NQ:
                proj(i + 1, wq_cur, wkv_cur)
            else:
                proj(0, wq_nxt, wkv_nxt, v_first=True)
            if i == 2:
                he = jnp.minimum(hn, H - 1)
                extract((he // HG) % 2, he % HG)
            if i == 4:
                gc = hn // HG + 1
                convert_slice(jnp.minimum(gc, NG - 1), gc % 2, hn % HG)
            softmax_pv(h, i, s_main, s_ext, tri)
        return carry

    def bprep_qkv(t, carry):
        c0 = pl.multiple_of(t * 128, 128)
        part = t // 8
        g = t % 8
        for mc in range(M // 128):
            blk = wqkv_s[mc * 128:(mc + 1) * 128, pl.ds(c0, 128)].astype(f32).T
            for h4 in range(4):
                tb[mc, pl.ds(h4, 32, stride=4), :] = blk[h4 * 32:(h4 + 1) * 32, :]
        for i in range(8):
            r0 = pl.multiple_of(part * 1024 + i * 128 + g * 16, 16)
            for mc in range(M // 128):
                wt_s[pl.ds(r0, 16), mc * 128:(mc + 1) * 128] = tb[mc, i * 16:(i + 1) * 16, :].astype(bf16)
        return carry

    def bprep_wo(g, carry):
        f0 = pl.multiple_of(g * 128, 128)
        for nc in range(M // 128):
            blk = wob_s[pl.ds(f0, 128), nc * 128:(nc + 1) * 128].astype(f32)
            for h4 in range(4):
                tb[nc, pl.ds(h4, 32, stride=4), :] = blk[h4 * 32:(h4 + 1) * 32, :]
        for i in range(8):
            r0 = pl.multiple_of(i * 128 + g * 16, 16)
            for nc in range(M // 128):
                wobp_s[pl.ds(r0, 16), nc * 128:(nc + 1) * 128] = tb[nc, i * 16:(i + 1) * 16, :].astype(bf16)
        return carry

    @pl.when(step == 0)
    def _phase1():
        g0 = cp_group(0)
        for cp in g0:
            cp.start()
        cp_c().start()
        cp_x().start()
        g1 = cp_group(1)
        for cp in g1:
            cp.start()
        kb_s[:, BR:BR + HALO, :] = jnp.zeros((8, HALO, 128), f32)
        vb_s[:, BR:BR + HALO, :] = jnp.zeros((8, HALO, 128), f32)
        for cp in g0:
            cp.wait()

        def conv0(sl, carry):
            convert_slice(0, 0, sl)
            return carry
        jax.lax.fori_loop(0, HG, conv0, 0)
        extract(0, 0)
        cp_c().wait()
        cp_x().wait()
        for g in range(2, NG):
            for cp in cp_group(g):
                cp.start()
        for cp in cp_rest():
            cp.start()
        proj(0, wq_nxt, wkv_nxt, v_first=True)
        for cp in g1:
            cp.wait()
        convert_slice(1, 1, 0)
        jax.lax.fori_loop(0, H, head_body, 0)
        for cp in cp_rest():
            cp.wait()
        jax.lax.fori_loop(0, 24, bprep_qkv, 0)
        jax.lax.fori_loop(0, 8, bprep_wo, 0)

    @pl.when(step > 0)
    def _phase2():
        t = step - 1
        r0 = pl.multiple_of(t * BR, BR)
        kb_s[:, 0:HALO, :] = kb_s[:, BR:BR + HALO, :]
        vb_s[:, 0:HALO, :] = vb_s[:, BR:BR + HALO, :]
        qkv = _dot_nt(xb_s[pl.ds(r0, BR), :], wt_s[...])
        for j in range(8):
            qb_s[j] = qkv[:, j * 128:(j + 1) * 128] * (BDH ** -0.5 * LOG2E)
            kb_s[j, HALO:HALO + BR, :] = qkv[:, 1024 + j * 128:1024 + (j + 1) * 128]
            vb_s[j, HALO:HALO + BR, :] = qkv[:, 2048 + j * 128:2048 + (j + 1) * 128]

        ctx = jnp.concatenate([ctx_s[h, pl.ds(r0, BR), :] for h in range(H)], axis=1)
        o_ref[:, 0:M] = _dot(ctx, wo_s[...]).astype(o_ref.dtype)

        lane = jax.lax.broadcasted_iota(jnp.int32, (CH, 128), 1)
        b2 = (lane & 4) != 0
        b3 = (lane & 8) != 0
        pos = jax.lax.broadcasted_iota(jnp.int32, (CH, 128), 0) + r0
        for cch in range(BR // CH):
            a0 = cch * CH
            logit = []
            for w in range(BW):
                acc = None
                for j in range(8):
                    term = qb_s[j, a0:a0 + CH, :] * kb_s[j, HALO + a0 - BDIL * w:HALO + a0 - BDIL * w + CH, :]
                    acc = term if acc is None else acc + term
                acc = acc + jnp.where(b2, pltpu.roll(acc, 4, 1), pltpu.roll(acc, 124, 1))
                acc = acc + jnp.where(b3, pltpu.roll(acc, 8, 1), pltpu.roll(acc, 120, 1))
                if cch == 0 and w > 0:
                    acc = jnp.where(pos >= BDIL * w, acc, NEG)
                logit.append(acc)
            mx = logit[0]
            for w in range(1, BW):
                mx = jnp.maximum(mx, logit[w])
            e = [jnp.exp2(lg - mx) for lg in logit]
            den = e[0]
            for w in range(1, BW):
                den = den + e[w]
            inv = _recip(den)
            e = [ew * inv for ew in e]
            for j in range(8):
                acc = None
                for w in range(BW):
                    term = e[w] * vb_s[j, HALO + a0 - BDIL * w:HALO + a0 - BDIL * w + CH, :]
                    acc = term if acc is None else acc + term
                ob_s[a0:a0 + CH, j * 128:(j + 1) * 128] = acc.astype(bf16)
        o_ref[:, M:2 * M] = _dot(ob_s[...], wobp_s[...]).astype(o_ref.dtype)


@jax.jit
def pallas_concat_heads__compressed_kv_cla__sliding_local_dilated__prompt_kernel(
    A_x: jax.Array,
    A_c_kv: jax.Array,
    A_w_q: jax.Array,
    A_w_uk: jax.Array,
    A_w_uv: jax.Array,
    A_w_o: jax.Array,
    B_x: jax.Array,
    B_wqkv: jax.Array,
    B_wo: jax.Array,
):
    x = A_x.reshape(S, M)
    c = A_c_kv.reshape(S, DC)
    wo = A_w_o.reshape(H * D, M)
    xb = B_x.reshape(S, M)

    any_spec = pl.BlockSpec(memory_space=pl.ANY)
    V = pltpu.VMEM
    scratch = [
        V((S, M), bf16),
        V((S, DC), bf16),
        V((NG, M, HG, D), bf16),
        V((NG, DC, HG, D), bf16),
        V((NG, DC, HG, D), bf16),
        V((2, M * HG, D), f32),
        V((2, DC * HG, D), f32),
        V((2, DC * HG, D), f32),
        V((M, D), bf16),
        V((DC, 2 * D), bf16),
        V((M, D), bf16),
        V((DC, 2 * D), bf16),
        V((S, D), bf16),
        V((S, D), bf16),
        V((S, D), bf16),
        V((BQ, D), bf16),
        V((H, S, D), bf16),
        V((H * D, M), bf16),
        V((S, M), bf16),
        V((M, 3 * M), bf16),
        V((M, M), bf16),
        V((3 * M, M), bf16),
        V((M, M), bf16),
        V((8, 128, 128), f32),
        V((8, BR, 128), f32),
        V((8, BR + HALO, 128), f32),
        V((8, BR + HALO, 128), f32),
        V((BR, M), bf16),
        pltpu.SemaphoreType.DMA((18,)),
    ]
    out = pl.pallas_call(
        _kernel,
        grid=(1 + NB,),
        in_specs=[any_spec] * 9,
        out_specs=pl.BlockSpec((BR, 2 * M), lambda s: (jnp.maximum(s - 1, 0), 0)),
        out_shape=jax.ShapeDtypeStruct((S, 2 * M), bf16),
        scratch_shapes=scratch,
        compiler_params=pltpu.CompilerParams(
            dimension_semantics=("arbitrary",),
            vmem_limit_bytes=120 * 1024 * 1024,
        ),
        name="fused_mla_local",
    )(x, c, A_w_q, A_w_uk, A_w_uv, wo, xb, B_wqkv, B_wo)
    return out.reshape(1, S, 2 * M)
```

```python
import jax
import jax.numpy as jnp
import jax.experimental.pallas as pl
import jax.experimental.pallas.tpu as pltpu

bf16 = jnp.bfloat16
f32 = jnp.float32

S = 2048
H = 32
D = 128
M = 1024
DC = 512
HG = 8
NG = H // HG
BQ = 256
NQ = S // BQ
HB = 128
BW = 8
BDIL = 2
BH = 32
BDH = 32
HALO = 16
BR = 256
NB = S // BR
CH = 32
LOG2E = 1.4426950408889634
NEG = -1e30
NT = (((1,), (1,)), ((), ()))
WT_BASE = (H + 1) * S
WOB_BASE = WT_BASE + 8 * 3 * M
POOL_ROWS = WOB_BASE + 8 * M
NWQ = 24


def _dot(a, b):
    return jnp.dot(a, b, preferred_element_type=f32)


def _dot_nt(a, b):
    return jax.lax.dot_general(a, b, NT, preferred_element_type=f32)


def _recip(x):
    r = pl.reciprocal(x, approx=True)
    return r * (2.0 - x * r)


def _kernel(x_hbm, c_hbm, wq_hbm, wuk_hbm, wuv_hbm, wo_hbm, xb_hbm, wqkv_hbm, wob_hbm,
            o_ref,
            x_s, c_s, rawq, rawk, rawv, tq, tk, tv,
            wq_cur, wkv_cur, wq_nxt, wkv_nxt,
            ka, va, vn, big, wo_s, xb_s, wqkv_s, wob_s,
            tb, qb_s, kb_s, vb_s, ob_s, sems):
    step = pl.program_id(0)
    zz = step

    SEM_X, SEM_C, SEM_Q, SEM_K, SEM_V = 0, 1, 2, 6, 10
    SEM_WO, SEM_XB, SEM_WOB, SEM_WQKV = 14, 15, 16, 17

    def cp_x():
        return pltpu.make_async_copy(x_hbm, x_s, sems.at[SEM_X])

    def cp_c():
        return pltpu.make_async_copy(c_hbm, c_s, sems.at[SEM_C])

    def cp_group(g, src_g=None):
        sg = g if src_g is None else src_g
        return [
            pltpu.make_async_copy(wq_hbm.at[:, pl.ds(sg * HG, HG), :], rawq.at[g], sems.at[SEM_Q + g]),
            pltpu.make_async_copy(wuk_hbm.at[:, pl.ds(sg * HG, HG), :], rawk.at[g], sems.at[SEM_K + g]),
            pltpu.make_async_copy(wuv_hbm.at[:, pl.ds(sg * HG, HG), :], rawv.at[g], sems.at[SEM_V + g]),
        ]

    def cp_wqkv(t, src_t=None):
        st = t if src_t is None else src_t
        return pltpu.make_async_copy(wqkv_hbm.at[:, pl.ds(st * 128, 128)], wqkv_s.at[t], sems.at[SEM_WQKV + t])

    def cp_rest():
        return [
            pltpu.make_async_copy(wob_hbm, wob_s, sems.at[SEM_WOB]),
            pltpu.make_async_copy(wo_hbm, wo_s, sems.at[SEM_WO]),
            pltpu.make_async_copy(xb_hbm, xb_s, sems.at[SEM_XB]),
        ]

    def rows(start, size, align):
        return pl.ds(pl.multiple_of(start, align), size)

    def convert_slice(g, par, sl):
        mq = M // HG
        m0 = pl.multiple_of(sl * mq, mq)
        tq[par, pl.ds(m0 * HG, mq * HG), :] = (
            rawq[g, pl.ds(m0, mq)].astype(f32).reshape(mq * HG, D))
        mk = DC // HG
        k0 = pl.multiple_of(sl * mk, mk)
        tk[par, pl.ds(k0 * HG, mk * HG), :] = (
            rawk[g, pl.ds(k0, mk)].astype(f32).reshape(mk * HG, D))
        tv[par, pl.ds(k0 * HG, mk * HG), :] = (
            rawv[g, pl.ds(k0, mk)].astype(f32).reshape(mk * HG, D))

    def extract(par, j):
        wq_nxt[...] = tq[par, pl.ds(j, M, stride=HG), :].astype(bf16)
        wkv_nxt[:, 0:D] = tk[par, pl.ds(j, DC, stride=HG), :].astype(bf16)
        wkv_nxt[:, D:2 * D] = tv[par, pl.ds(j, DC, stride=HG), :].astype(bf16)

    def proj(h, i, wq, wkv, staged):
        r = slice(i * BQ, (i + 1) * BQ)
        q = _dot(x_s[r, :], wq[...])
        big[rows((h + zz) * S + i * BQ, BQ, BQ), :] = (q * (D ** -0.5 * LOG2E)).astype(bf16)
        kv = _dot(c_s[r, :], wkv[...])
        ka[r, :] = kv[:, :D].astype(bf16)
        if staged:
            vn[r, :] = kv[:, D:].astype(bf16)
        else:
            va[r, :] = kv[:, D:].astype(bf16)

    def qk(h, i):
        r0 = i * BQ
        q = big[rows((h + zz) * S + r0, BQ, BQ), :]
        s_main = _dot_nt(q, ka[0:r0 + HB, :])
        q_lo = big[rows((h + zz) * S + r0 + HB, HB, HB), :]
        s_ext = _dot_nt(q_lo, ka[r0 + HB:r0 + BQ, :])
        return s_main, s_ext

    def softmax_pv(h, i, s_main, s_ext, tri, vr):
        r0 = i * BQ
        nt = 2 * i + 1
        tiles = [s_main[:, t * HB:(t + 1) * HB] for t in range(nt)]
        last = tiles[-1]
        tiles[-1] = jnp.concatenate([jnp.where(tri, last[:HB], NEG), last[HB:]], axis=0)
        ext = jnp.where(tri, s_ext, NEG)
        mt = tiles[0]
        for t in range(1, nt):
            mt = jnp.maximum(mt, tiles[t])
        mt = jnp.concatenate([mt[:HB], jnp.maximum(mt[HB:], ext)], axis=0)
        m = jnp.max(mt, axis=1, keepdims=True)
        pe = jnp.exp2(ext - m[HB:])
        ps = [jnp.exp2(tiles[t] - m) for t in range(nt)]
        p_main = jnp.concatenate(ps, axis=1).astype(bf16)
        lt = ps[0]
        for p in ps[1:]:
            lt = lt + p
        cm = _dot(p_main, vr[0:r0 + HB, :])
        lt = jnp.concatenate([lt[:HB], lt[HB:] + pe], axis=0)
        l = jnp.sum(lt, axis=1, keepdims=True)
        ce = _dot(pe.astype(bf16), vr[r0 + HB:r0 + BQ, :])
        cm = jnp.concatenate([cm[:HB], cm[HB:] + ce], axis=0)
        val = (cm * _recip(l)).astype(bf16)

        def store():
            big[rows(h * S + r0, BQ, BQ), :] = val
        return store

    def causal_tri():
        row = jax.lax.broadcasted_iota(jnp.int32, (HB, HB), 0)
        col = jax.lax.broadcasted_iota(jnp.int32, (HB, HB), 1)
        return col <= row

    def bprep_qkv(t):
        part = t // 8
        g = t % 8
        for mc in range(M // 128):
            blk = wqkv_s[t, mc * 128:(mc + 1) * 128, :].astype(f32).T
            for h4 in range(4):
                tb[mc, pl.ds(h4, 32, stride=4), :] = blk[h4 * 32:(h4 + 1) * 32, :]
        for mc in range(M // 128):
            for i in range(8):
                r0 = WT_BASE + mc * 3 * M + part * M + i * 128 + g * 16
                big[rows(r0, 16, 16), :] = tb[mc, i * 16:(i + 1) * 16, :].astype(bf16)

    def bprep_wo(g, carry):
        f0 = pl.multiple_of(g * 128, 128)
        for nc in range(M // 128):
            blk = wob_s[pl.ds(f0, 128), nc * 128:(nc + 1) * 128].astype(f32)
            for h4 in range(4):
                tb[nc, pl.ds(h4, 32, stride=4), :] = blk[h4 * 32:(h4 + 1) * 32, :]
        for nc in range(M // 128):
            for i in range(8):
                r0 = WOB_BASE + nc * M + i * 128 + g * 16
                big[rows(r0, 16, 16), :] = tb[nc, i * 16:(i + 1) * 16, :].astype(bf16)
        return carry

    def head_body(h, carry):
        hn = h + 1

        @pl.when(jnp.logical_and(hn % HG == 0, hn // HG + 1 < NG))
        def _():
            for cp in cp_group(hn // HG + 1, 0):
                cp.wait()

        @pl.when(jnp.logical_and(h >= 1, h < NWQ))
        def _():
            cp_wqkv(h, 0).wait()

        tri = causal_tri()
        va[0:2 * BQ, :] = vn[...]
        wq_cur[...] = wq_nxt[...]
        wkv_cur[...] = wkv_nxt[...]
        seq = [(h, i, va) for i in range(1, NQ)] + [(hn, 0, vn)]
        pend = []
        for hh, i, vr in seq:
            s_main, s_ext = qk(hh, i)
            if hh is hn:
                proj(hn, 1, wq_nxt, wkv_nxt, True)
            elif i + 1 == NQ:
                proj(hn, 0, wq_nxt, wkv_nxt, True)
            elif i == 1:
                proj(h, 2, wq_nxt, wkv_nxt, False)
            else:
                proj(h, i + 1, wq_cur, wkv_cur, False)
            if hh is h and i == 3:
                gc = hn // HG + 1
                convert_slice(jnp.minimum(gc, NG - 1), gc % 2, hn % HG)
                he = jnp.minimum(hn, H - 1)
                extract((he // HG) % 2, he % HG)
            if hh is h and i == 5:
                bprep_qkv(jnp.minimum(h, NWQ - 1))
            while len(pend) >= 2:
                pend.pop(0)()
            pend.append(softmax_pv(hh, i, s_main, s_ext, tri, vr))
        for st in pend:
            st()
        return carry

    @pl.when(step == 0)
    def _phase1():
        g0 = cp_group(0)
        for cp in g0:
            cp.start()
        cp_c().start()
        cp_x().start()
        g1 = cp_group(1)
        for cp in g1:
            cp.start()
        cp_wqkv(0).start()
        kb_s[:, BR:BR + HALO, :] = jnp.zeros((8, HALO, 128), f32)
        vb_s[:, BR:BR + HALO, :] = jnp.zeros((8, HALO, 128), f32)
        for cp in g0:
            cp.wait()

        def conv0(sl, carry):
            convert_slice(0, 0, sl)
            return carry
        jax.lax.fori_loop(0, HG, conv0, 0)
        extract(0, 0)
        cp_c().wait()
        cp_x().wait()
        for t in range(1, NWQ):
            cp_wqkv(t).start()
        for g in range(2, NG):
            for cp in cp_group(g):
                cp.start()
        for cp in cp_rest():
            cp.start()
        proj(0, 0, wq_nxt, wkv_nxt, True)
        s_main, s_ext = qk(0, 0)
        proj(0, 1, wq_nxt, wkv_nxt, True)
        softmax_pv(0, 0, s_main, s_ext, causal_tri(), vn)()
        for cp in g1:
            cp.wait()
        convert_slice(1, 1, 0)
        cp_wqkv(0).wait()
        jax.lax.fori_loop(0, H, head_body, 0)
        for cp in cp_rest():
            cp.wait()
        jax.lax.fori_loop(0, 8, bprep_wo, 0)

    @pl.when(step > 0)
    def _phase2():
        t = step - 1
        r0 = pl.multiple_of(t * BR, BR)
        kb_s[:, 0:HALO, :] = kb_s[:, BR:BR + HALO, :]
        vb_s[:, 0:HALO, :] = vb_s[:, BR:BR + HALO, :]
        wt = jnp.concatenate(
            [big[WT_BASE + mc * 3 * M:WT_BASE + (mc + 1) * 3 * M, :] for mc in range(8)], axis=1)
        qkv = _dot_nt(xb_s[pl.ds(r0, BR), :], wt)
        for j in range(8):
            qb_s[j] = qkv[:, j * 128:(j + 1) * 128] * (BDH ** -0.5 * LOG2E)
            kb_s[j, HALO:HALO + BR, :] = qkv[:, 1024 + j * 128:1024 + (j + 1) * 128]
            vb_s[j, HALO:HALO + BR, :] = qkv[:, 2048 + j * 128:2048 + (j + 1) * 128]

        ctx = jnp.concatenate([big[rows(h * S + r0, BR, BR), :] for h in range(H)], axis=1)
        o_ref[:, 0:M] = _dot(ctx, wo_s[...]).astype(o_ref.dtype)

        lane = jax.lax.broadcasted_iota(jnp.int32, (CH, 128), 1)
        b2 = (lane & 4) != 0
        b3 = (lane & 8) != 0
        pos = jax.lax.broadcasted_iota(jnp.int32, (CH, 128), 0) + r0
        for cch in range(BR // CH):
            a0 = cch * CH
            logit = []
            for w in range(BW):
                acc = None
                for j in range(8):
                    term = qb_s[j, a0:a0 + CH, :] * kb_s[j, HALO + a0 - BDIL * w:HALO + a0 - BDIL * w + CH, :]
                    acc = term if acc is None else acc + term
                acc = acc + jnp.where(b2, pltpu.roll(acc, 4, 1), pltpu.roll(acc, 124, 1))
                acc = acc + jnp.where(b3, pltpu.roll(acc, 8, 1), pltpu.roll(acc, 120, 1))
                if cch == 0 and w > 0:
                    acc = jnp.where(pos >= BDIL * w, acc, NEG)
                logit.append(acc)
            mx = logit[0]
            for w in range(1, BW):
                mx = jnp.maximum(mx, logit[w])
            e = [jnp.exp2(lg - mx) for lg in logit]
            den = e[0]
            for w in range(1, BW):
                den = den + e[w]
            inv = _recip(den)
            e = [ew * inv for ew in e]
            for j in range(8):
                acc = None
                for w in range(BW):
                    term = e[w] * vb_s[j, HALO + a0 - BDIL * w:HALO + a0 - BDIL * w + CH, :]
                    acc = term if acc is None else acc + term
                ob_s[a0:a0 + CH, j * 128:(j + 1) * 128] = acc.astype(bf16)
        wob = jnp.concatenate(
            [big[WOB_BASE + nc * M:WOB_BASE + (nc + 1) * M, :] for nc in range(8)], axis=1)
        o_ref[:, M:2 * M] = _dot(ob_s[...], wob).astype(o_ref.dtype)


@jax.jit
def pallas_concat_heads__compressed_kv_cla__sliding_local_dilated__prompt_kernel(
    A_x: jax.Array,
    A_c_kv: jax.Array,
    A_w_q: jax.Array,
    A_w_uk: jax.Array,
    A_w_uv: jax.Array,
    A_w_o: jax.Array,
    B_x: jax.Array,
    B_wqkv: jax.Array,
    B_wo: jax.Array,
):
    x = A_x.reshape(S, M)
    c = A_c_kv.reshape(S, DC)
    wo = A_w_o.reshape(H * D, M)
    xb = B_x.reshape(S, M)

    any_spec = pl.BlockSpec(memory_space=pl.ANY)
    V = pltpu.VMEM
    scratch = [
        V((S, M), bf16),
        V((S, DC), bf16),
        V((NG, M, HG, D), bf16),
        V((NG, DC, HG, D), bf16),
        V((NG, DC, HG, D), bf16),
        V((2, M * HG, D), f32),
        V((2, DC * HG, D), f32),
        V((2, DC * HG, D), f32),
        V((M, D), bf16),
        V((DC, 2 * D), bf16),
        V((M, D), bf16),
        V((DC, 2 * D), bf16),
        V((S, D), bf16),
        V((S, D), bf16),
        V((2 * BQ, D), bf16),
        V((POOL_ROWS, D), bf16),
        V((H * D, M), bf16),
        V((S, M), bf16),
        V((NWQ, M, 128), bf16),
        V((M, M), bf16),
        V((8, 128, 128), f32),
        V((8, BR, 128), f32),
        V((8, BR + HALO, 128), f32),
        V((8, BR + HALO, 128), f32),
        V((BR, M), bf16),
        pltpu.SemaphoreType.DMA((17 + NWQ,)),
    ]
    out = pl.pallas_call(
        _kernel,
        grid=(1 + NB,),
        in_specs=[any_spec] * 9,
        out_specs=pl.BlockSpec((BR, 2 * M), lambda s: (jnp.maximum(s - 1, 0), 0)),
        out_shape=jax.ShapeDtypeStruct((S, 2 * M), bf16),
        scratch_shapes=scratch,
        compiler_params=pltpu.CompilerParams(
            dimension_semantics=("arbitrary",),
            vmem_limit_bytes=120 * 1024 * 1024,
        ),
        name="fused_mla_local",
    )(x, c, A_w_q, A_w_uk, A_w_uv, wo, xb, B_wqkv, B_wo)
    return out.reshape(1, S, 2 * M)
```

```python
import jax
import jax.numpy as jnp
import jax.experimental.pallas as pl
import jax.experimental.pallas.tpu as pltpu

bf16 = jnp.bfloat16
f32 = jnp.float32

S = 2048
H = 32
D = 128
M = 1024
DC = 512
HG = 8
NG = H // HG
BQ = 256
NQ = S // BQ
HB = 128
BW = 8
BDIL = 2
BH = 32
BDH = 32
HALO = 16
BR = 256
NB = S // BR
CH = 8
KS = 4
LOG2E = 1.4426950408889634
NEG = -1e30
NT = (((1,), (1,)), ((), ()))
WT_BASE = (H + 1) * S
WOB_BASE = WT_BASE + 8 * 3 * M
POOL_ROWS = WOB_BASE + 8 * M
NWQ = 24


def _dot(a, b):
    return jnp.dot(a, b, preferred_element_type=f32)


def _dot_nt(a, b):
    return jax.lax.dot_general(a, b, NT, preferred_element_type=f32)


def _recip(x):
    r = pl.reciprocal(x, approx=True)
    return r * (2.0 - x * r)


def _kernel(x_hbm, c_hbm, wq_hbm, wuk_hbm, wuv_hbm, wo_hbm, xb_hbm, wqkv_hbm, wob_hbm,
            o_ref,
            x_s, c_s, rawq, rawk, rawv, tq, tk, tv,
            wq_cur, wkv_cur, wq_nxt, wkv_nxt,
            ka, va, vn, big, wo_s, xb_s, wqkv_s, wob_s,
            tb, qb_s, kb_s, vb_s, ob_s, zero_s, sems):
    step = pl.program_id(0)
    zz = step

    SEM_G0, SEM_XC, SEM_SET, SEM_REST = 0, 4, 6, 10
    MQ, MK = M // HG, DC // HG

    def cp_slices(g, s0, n, sem):
        heads = pl.ds(g * HG, HG)
        return [
            pltpu.make_async_copy(wuk_hbm.at[pl.ds(s0 * MK, n * MK), heads, :], rawk.at[g, pl.ds(s0 * MK, n * MK)], sem),
            pltpu.make_async_copy(wuv_hbm.at[pl.ds(s0 * MK, n * MK), heads, :], rawv.at[g, pl.ds(s0 * MK, n * MK)], sem),
            pltpu.make_async_copy(wq_hbm.at[pl.ds(s0 * MQ, n * MQ), heads, :], rawq.at[g, pl.ds(s0 * MQ, n * MQ)], sem),
        ]

    def cp_g0(k):
        return cp_slices(0, 2 * k, 2, sems.at[SEM_G0 + k])

    def cp_xc(k):
        r = pl.ds(0, 2 * BQ) if k == 0 else pl.ds(2 * BQ, S - 2 * BQ)
        return [
            pltpu.make_async_copy(c_hbm.at[r], c_s.at[r], sems.at[SEM_XC + k]),
            pltpu.make_async_copy(x_hbm.at[r], x_s.at[r], sems.at[SEM_XC + k]),
        ]

    SETS = ((1, 0, 1, 0, 1), (1, 1, 7, 1, 7), (2, 0, 8, 8, 8), (3, 0, 8, 16, 8))
    SET_BODY = (0, 1, 8, 16)

    def cp_set(k):
        g, s0, n, t0, nt = SETS[k]
        sem = sems.at[SEM_SET + k]
        cols = pl.ds(t0 * 128, nt * 128)
        return cp_slices(g, s0, n, sem) + [pltpu.make_async_copy(wqkv_hbm.at[:, cols], wqkv_s.at[:, cols], sem)]

    def cp_rest():
        return [
            pltpu.make_async_copy(wob_hbm, wob_s, sems.at[SEM_REST]),
            pltpu.make_async_copy(xb_hbm, xb_s, sems.at[SEM_REST + 1]),
            pltpu.make_async_copy(wo_hbm, wo_s, sems.at[SEM_REST + 2]),
        ]

    def start(cps):
        for cp in cps:
            cp.start()

    def wait(cps):
        for cp in cps:
            cp.wait()

    def rows(start, size, align):
        return pl.ds(start if isinstance(start, int) else pl.multiple_of(start, align), size)

    def convert_slice(g, par, sl):
        mq = M // HG
        m0 = sl * mq if isinstance(sl, int) else pl.multiple_of(sl * mq, mq)
        tq[par, pl.ds(m0 * HG, mq * HG), :] = (
            rawq[g, pl.ds(m0, mq)].astype(f32).reshape(mq * HG, D))
        mk = DC // HG
        k0 = sl * mk if isinstance(sl, int) else pl.multiple_of(sl * mk, mk)
        tk[par, pl.ds(k0 * HG, mk * HG), :] = (
            rawk[g, pl.ds(k0, mk)].astype(f32).reshape(mk * HG, D))
        tv[par, pl.ds(k0 * HG, mk * HG), :] = (
            rawv[g, pl.ds(k0, mk)].astype(f32).reshape(mk * HG, D))

    def extract(par, j):
        wq_nxt[...] = tq[par, pl.ds(j, M, stride=HG), :].astype(bf16)
        wkv_nxt[:, 0:D] = tk[par, pl.ds(j, DC, stride=HG), :].astype(bf16)
        wkv_nxt[:, D:2 * D] = tv[par, pl.ds(j, DC, stride=HG), :].astype(bf16)

    def proj(h, i, wq, wkv, staged):
        r = slice(i * BQ, (i + 1) * BQ)
        q = _dot(x_s[r, :], wq[...])
        big[rows((h + zz) * S + i * BQ, BQ, BQ), :] = (q * (D ** -0.5 * LOG2E)).astype(bf16)
        kv = _dot(c_s[r, :], wkv[...])
        ka[r, :] = kv[:, :D].astype(bf16)
        if staged:
            vn[r, :] = kv[:, D:].astype(bf16)
        else:
            va[r, :] = kv[:, D:].astype(bf16)

    def qk(h, i):
        r0 = i * BQ
        q = big[rows((h + zz) * S + r0, BQ, BQ), :]
        s_main = _dot_nt(q, ka[0:r0 + HB, :])
        q_lo = big[rows((h + zz) * S + r0 + HB, HB, HB), :]
        s_ext = _dot_nt(q_lo, ka[r0 + HB:r0 + BQ, :])
        return s_main, s_ext

    def softmax_pv(h, i, s_main, s_ext, tri, vr):
        r0 = i * BQ
        nt = 2 * i + 1
        tiles = [s_main[:, t * HB:(t + 1) * HB] for t in range(nt)]
        last = tiles[-1]
        tiles[-1] = jnp.concatenate([jnp.where(tri, last[:HB], NEG), last[HB:]], axis=0)
        ext = jnp.where(tri, s_ext, NEG)
        mt = tiles[0]
        for t in range(1, nt):
            mt = jnp.maximum(mt, tiles[t])
        mt = jnp.concatenate([mt[:HB], jnp.maximum(mt[HB:], ext)], axis=0)
        m = jnp.max(mt, axis=1, keepdims=True)
        pe = jnp.exp2(ext - m[HB:])
        ps = [jnp.exp2(tiles[t] - m) for t in range(nt)]
        p_main = jnp.concatenate(ps, axis=1).astype(bf16)
        lt = ps[0]
        for p in ps[1:]:
            lt = lt + p
        cm = _dot(p_main, vr[0:r0 + HB, :])
        lt = jnp.concatenate([lt[:HB], lt[HB:] + pe], axis=0)
        l = jnp.sum(lt, axis=1, keepdims=True)
        ce = _dot(pe.astype(bf16), vr[r0 + HB:r0 + BQ, :])
        cm = jnp.concatenate([cm[:HB], cm[HB:] + ce], axis=0)
        val = (cm * _recip(l)).astype(bf16)

        def store():
            big[rows(h * S + r0, BQ, BQ), :] = val
        return store

    def causal_tri():
        row = jax.lax.broadcasted_iota(jnp.int32, (HB, HB), 0)
        col = jax.lax.broadcasted_iota(jnp.int32, (HB, HB), 1)
        return col <= row

    def bprep_qkv(t):
        part = t // 8
        g = t % 8
        for mc in range(M // 128):
            blk = wqkv_s[mc * 128:(mc + 1) * 128, pl.ds(pl.multiple_of(t * 128, 128), 128)].astype(f32).T
            for h4 in range(4):
                tb[mc, pl.ds(h4, 32, stride=4), :] = blk[h4 * 32:(h4 + 1) * 32, :]
        for mc in range(M // 128):
            for i in range(8):
                r0 = WT_BASE + mc * 3 * M + part * M + i * 128 + g * 16
                big[rows(r0, 16, 16), :] = tb[mc, i * 16:(i + 1) * 16, :].astype(bf16)

    def bprep_wo(g, carry):
        f0 = pl.multiple_of(g * 128, 128)
        for nc in range(M // 128):
            blk = wob_s[pl.ds(f0, 128), nc * 128:(nc + 1) * 128].astype(f32)
            for h4 in range(4):
                tb[nc, pl.ds(h4, 32, stride=4), :] = blk[h4 * 32:(h4 + 1) * 32, :]
        for nc in range(M // 128):
            for i in range(8):
                r0 = WOB_BASE + nc * M + i * 128 + g * 16
                big[rows(r0, 16, 16), :] = tb[nc, i * 16:(i + 1) * 16, :].astype(bf16)
        return carry

    def head_body(h, carry):
        hn = h + 1

        for k in range(1, len(SETS)):
            @pl.when(h == SET_BODY[k])
            def _():
                wait(cp_set(k))

        tri = causal_tri()
        va[0:2 * BQ, :] = vn[...]
        wq_cur[...] = wq_nxt[...]
        wkv_cur[...] = wkv_nxt[...]
        seq = [(h, i, va) for i in range(1, NQ)] + [(hn, 0, vn)]
        pend = []
        for hh, i, vr in seq:
            s_main, s_ext = qk(hh, i)
            if hh is hn:
                proj(hn, 1, wq_nxt, wkv_nxt, True)
            elif i + 1 == NQ:
                proj(hn, 0, wq_nxt, wkv_nxt, True)
            elif i == 1:
                proj(h, 2, wq_nxt, wkv_nxt, False)
            else:
                proj(h, i + 1, wq_cur, wkv_cur, False)
            if hh is h and i == 3:
                gc = h // HG + 1
                convert_slice(jnp.minimum(gc, NG - 1), gc % 2, h % HG)
                he = jnp.minimum(hn, H - 1)
                extract((he // HG) % 2, he % HG)
            if hh is h and i == 5:
                bprep_qkv(jnp.minimum(h, NWQ - 1))
            while len(pend) >= 2:
                pend.pop(0)()
            pend.append(softmax_pv(hh, i, s_main, s_ext, tri, vr))
        for st in pend:
            st()
        return carry

    def b_qkv(t):
        kb_s[:, 0:HALO, :] = kb_s[:, BR:BR + HALO, :]
        vb_s[:, 0:HALO, :] = vb_s[:, BR:BR + HALO, :]
        wt = jnp.concatenate(
            [big[WT_BASE + mc * 3 * M:WT_BASE + (mc + 1) * 3 * M, :] for mc in range(8)], axis=1)
        qkv = _dot_nt(xb_s[rows(t * BR, BR, BR), :], wt)
        for j in range(8):
            qb_s[j] = qkv[:, j * 128:(j + 1) * 128] * (BDH ** -0.5 * LOG2E)
            kb_s[j, HALO:HALO + BR, :] = qkv[:, 1024 + j * 128:1024 + (j + 1) * 128]
            vb_s[j, HALO:HALO + BR, :] = qkv[:, 2048 + j * 128:2048 + (j + 1) * 128]

    def b_attn_chunk(r0, cch, never, tok):
        a0 = cch * CH
        lane = jax.lax.broadcasted_iota(jnp.int32, (CH, 128), 1)
        b2 = (lane & 4) != 0
        b3 = (lane & 8) != 0
        qs = [qb_s[j, a0:a0 + CH, :] for j in range(8)]
        if tok is not None:
            qs = [jnp.where(never, tok, q) for q in qs]
        logit = []
        for w in range(BW):
            acc = None
            for j in range(8):
                term = qs[j] * kb_s[j, HALO + a0 - BDIL * w:HALO + a0 - BDIL * w + CH, :]
                acc = term if acc is None else acc + term
            acc = acc + jnp.where(b2, pltpu.roll(acc, 4, 1), pltpu.roll(acc, 124, 1))
            acc = acc + jnp.where(b3, pltpu.roll(acc, 8, 1), pltpu.roll(acc, 120, 1))
            if a0 < BDIL * w:
                pos = jax.lax.broadcasted_iota(jnp.int32, (CH, 128), 0) + (r0 + a0)
                acc = jnp.where(pos >= BDIL * w, acc, NEG)
            logit.append(acc)
        mx = logit[0]
        for w in range(1, BW):
            mx = jnp.maximum(mx, logit[w])
        e = [jnp.exp2(lg - mx) for lg in logit]
        den = e[0]
        for w in range(1, BW):
            den = den + e[w]
        inv = _recip(den)
        e = [ew * inv for ew in e]
        outs = []
        for j in range(8):
            acc = None
            for w in range(BW):
                term = e[w] * vb_s[j, HALO + a0 - BDIL * w:HALO + a0 - BDIL * w + CH, :]
                acc = term if acc is None else acc + term
            outs.append(acc)
        return outs

    @pl.when(step == 0)
    def _phase1():
        for k in range(HG // 2):
            start(cp_g0(k))
        start(cp_xc(0))
        start(cp_xc(1))
        for k in range(len(SETS)):
            start(cp_set(k))
        start(cp_rest())
        zero_s[0] = 0
        kb_s[:, BR:BR + HALO, :] = jnp.zeros((8, HALO, 128), f32)
        vb_s[:, BR:BR + HALO, :] = jnp.zeros((8, HALO, 128), f32)
        for k in range(HG // 2):
            wait(cp_g0(k))
            convert_slice(0, 0, 2 * k)
            convert_slice(0, 0, 2 * k + 1)
        extract(0, 0)
        wait(cp_xc(0))
        proj(0, 0, wq_nxt, wkv_nxt, True)
        s_main, s_ext = qk(0, 0)
        proj(0, 1, wq_nxt, wkv_nxt, True)
        softmax_pv(0, 0, s_main, s_ext, causal_tri(), vn)()
        wait(cp_xc(1))
        wait(cp_set(0))
        jax.lax.fori_loop(0, H, head_body, 0)
        wait(cp_rest())
        jax.lax.fori_loop(0, 8, bprep_wo, 0)

    @pl.when(step > 1)
    def _phase2():
        t = step - 2
        r0 = pl.multiple_of(t * BR, BR)
        never = zero_s[0] > 0
        ctx = jnp.concatenate([big[rows(h * S + r0, BR, BR), :] for h in range(H)], axis=1)
        nstage = (M // 128) * KS
        per = (BR // CH) // nstage
        kw = (H * D) // KS
        tok = None
        stage = 0
        half = []
        for p in range(M // 128):
            res = None
            for kk in range(KS):
                for cch in range(stage * per, (stage + 1) * per):
                    outs = b_attn_chunk(r0, cch, never, tok)
                    half.append(outs)
                    if len(half) * CH == 16:
                        a0 = (cch + 1) * CH - 16
                        for j in range(8):
                            ob_s[a0:a0 + 16, j * 128:(j + 1) * 128] = jnp.concatenate(
                                [hf[j] for hf in half], axis=0).astype(bf16)
                        half = []
                part = _dot(ctx[:, kk * kw:(kk + 1) * kw], wo_s[kk * kw:(kk + 1) * kw, p * 128:(p + 1) * 128])
                res = part if res is None else res + part
                tok = res[0:CH, :]
                stage += 1
            o_ref[:, p * 128:(p + 1) * 128] = res.astype(o_ref.dtype)
        wob = jnp.concatenate(
            [big[WOB_BASE + nc * M:WOB_BASE + (nc + 1) * M, :] for nc in range(8)], axis=1)
        o_ref[:, M:2 * M] = _dot(ob_s[...], wob).astype(o_ref.dtype)

    @pl.when(jnp.logical_and(step >= 1, step <= NB))
    def _phase2_qkv():
        b_qkv(step - 1)


@jax.jit
def pallas_concat_heads__compressed_kv_cla__sliding_local_dilated__prompt_kernel(
    A_x: jax.Array,
    A_c_kv: jax.Array,
    A_w_q: jax.Array,
    A_w_uk: jax.Array,
    A_w_uv: jax.Array,
    A_w_o: jax.Array,
    B_x: jax.Array,
    B_wqkv: jax.Array,
    B_wo: jax.Array,
):
    x = A_x.reshape(S, M)
    c = A_c_kv.reshape(S, DC)
    wo = A_w_o.reshape(H * D, M)
    xb = B_x.reshape(S, M)

    any_spec = pl.BlockSpec(memory_space=pl.ANY)
    V = pltpu.VMEM
    scratch = [
        V((S, M), bf16),
        V((S, DC), bf16),
        V((NG, M, HG, D), bf16),
        V((NG, DC, HG, D), bf16),
        V((NG, DC, HG, D), bf16),
        V((2, M * HG, D), f32),
        V((2, DC * HG, D), f32),
        V((2, DC * HG, D), f32),
        V((M, D), bf16),
        V((DC, 2 * D), bf16),
        V((M, D), bf16),
        V((DC, 2 * D), bf16),
        V((S, D), bf16),
        V((S, D), bf16),
        V((2 * BQ, D), bf16),
        V((POOL_ROWS, D), bf16),
        V((H * D, M), bf16),
        V((S, M), bf16),
        V((M, 3 * M), bf16),
        V((M, M), bf16),
        V((8, 128, 128), f32),
        V((8, BR, 128), f32),
        V((8, BR + HALO, 128), f32),
        V((8, BR + HALO, 128), f32),
        V((BR, M), bf16),
        pltpu.SMEM((1,), jnp.int32),
        pltpu.SemaphoreType.DMA((13,)),
    ]
    out = pl.pallas_call(
        _kernel,
        grid=(2 + NB,),
        in_specs=[any_spec] * 9,
        out_specs=pl.BlockSpec((BR, 2 * M), lambda s: (jnp.maximum(s - 2, 0), 0)),
        out_shape=jax.ShapeDtypeStruct((S, 2 * M), bf16),
        scratch_shapes=scratch,
        compiler_params=pltpu.CompilerParams(
            dimension_semantics=("arbitrary",),
            vmem_limit_bytes=120 * 1024 * 1024,
            disable_bounds_checks=True,
        ),
        name="fused_mla_local",
    )(x, c, A_w_q, A_w_uk, A_w_uv, wo, xb, B_wqkv, B_wo)
    return out.reshape(1, S, 2 * M)
```

```python
import jax
import jax.numpy as jnp
import jax.experimental.pallas as pl
import jax.experimental.pallas.tpu as pltpu

bf16 = jnp.bfloat16
f32 = jnp.float32

S = 2048
H = 32
D = 128
M = 1024
DC = 512
HG = 8
NG = H // HG
BQ = 256
NQ = S // BQ
HB = 128
BW = 8
BDIL = 2
BH = 32
BDH = 32
HALO = 16
BR = 256
NB = S // BR
CH = 8
KS = 4
LOG2E = 1.4426950408889634
NEG = -1e30
NT = (((1,), (1,)), ((), ()))
WT_BASE = (H + 1) * S
WOB_BASE = WT_BASE + 8 * 3 * M
POOL_ROWS = WOB_BASE + 8 * M
NWQ = 24
CONV_AT = 2
EXT_AT = 2
BPREP_AT = 4


def _dot(a, b):
    return jnp.dot(a, b, preferred_element_type=f32)


def _dot_nt(a, b):
    return jax.lax.dot_general(a, b, NT, preferred_element_type=f32)


def _recip(x):
    r = pl.reciprocal(x, approx=True)
    return r * (2.0 - x * r)


def _kernel(x_hbm, c_hbm, wq_hbm, wuk_hbm, wuv_hbm, wo_hbm, xb_hbm, wqkv_hbm, wob_hbm,
            o_ref,
            x_s, c_s, rawq, rawk, rawv, tq, tk, tv,
            wbuf,
            ka, va, vn, big, wo_s, xb_s, wqkv_s, wob_s,
            tb, qb_s, kb_s, vb_s, ob_s, zero_s, sems):
    step = pl.program_id(0)
    zz = step

    SEM_G0, SEM_XC, SEM_SET, SEM_REST = 0, 4, 6, 10
    MQ, MK = M // HG, DC // HG

    def cp_slices(g, s0, n, sem):
        heads = pl.ds(g * HG, HG)
        return [
            pltpu.make_async_copy(wuk_hbm.at[pl.ds(s0 * MK, n * MK), heads, :], rawk.at[g, pl.ds(s0 * MK, n * MK)], sem),
            pltpu.make_async_copy(wuv_hbm.at[pl.ds(s0 * MK, n * MK), heads, :], rawv.at[g, pl.ds(s0 * MK, n * MK)], sem),
            pltpu.make_async_copy(wq_hbm.at[pl.ds(s0 * MQ, n * MQ), heads, :], rawq.at[g, pl.ds(s0 * MQ, n * MQ)], sem),
        ]

    def cp_g0(k):
        return cp_slices(0, 2 * k, 2, sems.at[SEM_G0 + k])

    def cp_xc(k):
        r = pl.ds(0, 2 * BQ) if k == 0 else pl.ds(2 * BQ, S - 2 * BQ)
        return [
            pltpu.make_async_copy(c_hbm.at[r], c_s.at[r], sems.at[SEM_XC + k]),
            pltpu.make_async_copy(x_hbm.at[r], x_s.at[r], sems.at[SEM_XC + k]),
        ]

    SETS = ((1, 0, 1, 0, 1), (1, 1, 7, 1, 7), (2, 0, 8, 8, 8), (3, 0, 8, 16, 8))
    SET_BODY = (0, 1, 8, 16)

    def cp_set(k):
        g, s0, n, t0, nt = SETS[k]
        sem = sems.at[SEM_SET + k]
        cols = pl.ds(t0 * 128, nt * 128)
        return cp_slices(g, s0, n, sem) + [pltpu.make_async_copy(wqkv_hbm.at[:, cols], wqkv_s.at[:, cols], sem)]

    def cp_rest():
        return [
            pltpu.make_async_copy(wob_hbm, wob_s, sems.at[SEM_REST]),
            pltpu.make_async_copy(xb_hbm, xb_s, sems.at[SEM_REST + 1]),
            pltpu.make_async_copy(wo_hbm, wo_s, sems.at[SEM_REST + 2]),
        ]

    def start(cps):
        for cp in cps:
            cp.start()

    def wait(cps):
        for cp in cps:
            cp.wait()

    def rows(start, size, align):
        return pl.ds(start if isinstance(start, int) else pl.multiple_of(start, align), size)

    def convert_slice(g, par, sl):
        mq = M // HG
        m0 = sl * mq if isinstance(sl, int) else pl.multiple_of(sl * mq, mq)
        tq[par, pl.ds(m0 * HG, mq * HG), :] = (
            rawq[g, pl.ds(m0, mq)].astype(f32).reshape(mq * HG, D))
        mk = DC // HG
        k0 = sl * mk if isinstance(sl, int) else pl.multiple_of(sl * mk, mk)
        tk[par, pl.ds(k0 * HG, mk * HG), :] = (
            rawk[g, pl.ds(k0, mk)].astype(f32).reshape(mk * HG, D))
        tv[par, pl.ds(k0 * HG, mk * HG), :] = (
            rawv[g, pl.ds(k0, mk)].astype(f32).reshape(mk * HG, D))

    def extract(par, j, wp):
        wbuf[wp, 0:M, :] = tq[par, pl.ds(j, M, stride=HG), :].astype(bf16)
        wbuf[wp, M:M + DC, :] = tk[par, pl.ds(j, DC, stride=HG), :].astype(bf16)
        wbuf[wp, M + DC:M + 2 * DC, :] = tv[par, pl.ds(j, DC, stride=HG), :].astype(bf16)

    def proj(h, i, staged):
        r = slice(i * BQ, (i + 1) * BQ)
        wp = h % 2
        q = _dot(x_s[r, :], wbuf[wp, 0:M, :])
        big[rows((h + zz) * S + i * BQ, BQ, BQ), :] = (q * (D ** -0.5 * LOG2E)).astype(bf16)
        wkv = jnp.concatenate([wbuf[wp, M:M + DC, :], wbuf[wp, M + DC:M + 2 * DC, :]], axis=1)
        kv = _dot(c_s[r, :], wkv)
        ka[r, :] = kv[:, :D].astype(bf16)
        if staged:
            vn[r, :] = kv[:, D:].astype(bf16)
        else:
            va[r, :] = kv[:, D:].astype(bf16)

    def qk(h, i):
        r0 = i * BQ
        q = big[rows((h + zz) * S + r0, BQ, BQ), :]
        s_main = _dot_nt(q, ka[0:r0 + HB, :])
        q_lo = big[rows((h + zz) * S + r0 + HB, HB, HB), :]
        s_ext = _dot_nt(q_lo, ka[r0 + HB:r0 + BQ, :])
        return s_main, s_ext

    def softmax_pv(h, i, s_main, s_ext, tri, vr):
        r0 = i * BQ
        nt = 2 * i + 1
        tiles = [s_main[:, t * HB:(t + 1) * HB] for t in range(nt)]
        last = tiles[-1]
        tiles[-1] = jnp.concatenate([jnp.where(tri, last[:HB], NEG), last[HB:]], axis=0)
        ext = jnp.where(tri, s_ext, NEG)
        mt = tiles[0]
        for t in range(1, nt):
            mt = jnp.maximum(mt, tiles[t])
        mt = jnp.concatenate([mt[:HB], jnp.maximum(mt[HB:], ext)], axis=0)
        m = jnp.max(mt, axis=1, keepdims=True)
        pe = jnp.exp2(ext - m[HB:])
        ps = [jnp.exp2(tiles[t] - m) for t in range(nt)]
        p_main = jnp.concatenate(ps, axis=1).astype(bf16)
        lt = ps[0]
        for p in ps[1:]:
            lt = lt + p
        cm = _dot(p_main, vr[0:r0 + HB, :])
        lt = jnp.concatenate([lt[:HB], lt[HB:] + pe], axis=0)
        l = jnp.sum(lt, axis=1, keepdims=True)
        ce = _dot(pe.astype(bf16), vr[r0 + HB:r0 + BQ, :])
        cm = jnp.concatenate([cm[:HB], cm[HB:] + ce], axis=0)
        val = (cm * _recip(l)).astype(bf16)

        def store():
            big[rows(h * S + r0, BQ, BQ), :] = val
        return store

    def causal_tri():
        row = jax.lax.broadcasted_iota(jnp.int32, (HB, HB), 0)
        col = jax.lax.broadcasted_iota(jnp.int32, (HB, HB), 1)
        return col <= row

    def bprep_qkv(t):
        part = t // 8
        g = t % 8
        for mc in range(M // 128):
            blk = wqkv_s[mc * 128:(mc + 1) * 128, pl.ds(pl.multiple_of(t * 128, 128), 128)].astype(f32).T
            for h4 in range(4):
                tb[mc, pl.ds(h4, 32, stride=4), :] = blk[h4 * 32:(h4 + 1) * 32, :]
        for mc in range(M // 128):
            for i in range(8):
                r0 = WT_BASE + mc * 3 * M + part * M + i * 128 + g * 16
                big[rows(r0, 16, 16), :] = tb[mc, i * 16:(i + 1) * 16, :].astype(bf16)

    def bprep_wo(g, carry):
        f0 = pl.multiple_of(g * 128, 128)
        for nc in range(M // 128):
            blk = wob_s[pl.ds(f0, 128), nc * 128:(nc + 1) * 128].astype(f32)
            for h4 in range(4):
                tb[nc, pl.ds(h4, 32, stride=4), :] = blk[h4 * 32:(h4 + 1) * 32, :]
        for nc in range(M // 128):
            for i in range(8):
                r0 = WOB_BASE + nc * M + i * 128 + g * 16
                big[rows(r0, 16, 16), :] = tb[nc, i * 16:(i + 1) * 16, :].astype(bf16)
        return carry

    def head_body(h, carry):
        hn = h + 1

        for k in range(1, len(SETS)):
            @pl.when(h == SET_BODY[k])
            def _():
                wait(cp_set(k))

        tri = causal_tri()
        va[0:2 * BQ, :] = vn[...]
        seq = [(h, i, va) for i in range(1, NQ)] + [(hn, 0, vn)]
        pend = []
        for hh, i, vr in seq:
            s_main, s_ext = qk(hh, i)
            if hh is hn:
                proj(hn, 1, True)
            elif i + 1 == NQ:
                proj(hn, 0, True)
            else:
                proj(h, i + 1, False)
            if hh is h and i == CONV_AT:
                gc = h // HG + 1
                convert_slice(jnp.minimum(gc, NG - 1), gc % 2, h % HG)
            if hh is h and i == EXT_AT:
                he = jnp.minimum(hn, H - 1)
                extract((he // HG) % 2, he % HG, hn % 2)
            if hh is h and i == BPREP_AT:
                bprep_qkv(jnp.minimum(h, NWQ - 1))
            while len(pend) >= 2:
                pend.pop(0)()
            pend.append(softmax_pv(hh, i, s_main, s_ext, tri, vr))
        for st in pend:
            st()
        return carry

    def b_qkv(t):
        kb_s[:, 0:HALO, :] = kb_s[:, BR:BR + HALO, :]
        vb_s[:, 0:HALO, :] = vb_s[:, BR:BR + HALO, :]
        wt = jnp.concatenate(
            [big[WT_BASE + mc * 3 * M:WT_BASE + (mc + 1) * 3 * M, :] for mc in range(8)], axis=1)
        qkv = _dot_nt(xb_s[rows(t * BR, BR, BR), :], wt)
        for j in range(8):
            qb_s[j] = qkv[:, j * 128:(j + 1) * 128] * (BDH ** -0.5 * LOG2E)
            kb_s[j, HALO:HALO + BR, :] = qkv[:, 1024 + j * 128:1024 + (j + 1) * 128]
            vb_s[j, HALO:HALO + BR, :] = qkv[:, 2048 + j * 128:2048 + (j + 1) * 128]

    def b_attn_chunk(r0, cch, never, tok):
        a0 = cch * CH
        lane = jax.lax.broadcasted_iota(jnp.int32, (CH, 128), 1)
        b2 = (lane & 4) != 0
        b3 = (lane & 8) != 0
        qs = [qb_s[j, a0:a0 + CH, :] for j in range(8)]
        if tok is not None:
            qs = [jnp.where(never, tok, q) for q in qs]
        logit = []
        for w in range(BW):
            acc = None
            for j in range(8):
                term = qs[j] * kb_s[j, HALO + a0 - BDIL * w:HALO + a0 - BDIL * w + CH, :]
                acc = term if acc is None else acc + term
            acc = acc + jnp.where(b2, pltpu.roll(acc, 4, 1), pltpu.roll(acc, 124, 1))
            acc = acc + jnp.where(b3, pltpu.roll(acc, 8, 1), pltpu.roll(acc, 120, 1))
            if a0 < BDIL * w:
                pos = jax.lax.broadcasted_iota(jnp.int32, (CH, 128), 0) + (r0 + a0)
                acc = jnp.where(pos >= BDIL * w, acc, NEG)
            logit.append(acc)
        mx = logit[0]
        for w in range(1, BW):
            mx = jnp.maximum(mx, logit[w])
        e = [jnp.exp2(lg - mx) for lg in logit]
        den = e[0]
        for w in range(1, BW):
            den = den + e[w]
        inv = _recip(den)
        e = [ew * inv for ew in e]
        outs = []
        for j in range(8):
            acc = None
            for w in range(BW):
                term = e[w] * vb_s[j, HALO + a0 - BDIL * w:HALO + a0 - BDIL * w + CH, :]
                acc = term if acc is None else acc + term
            outs.append(acc)
        return outs

    @pl.when(step == 0)
    def _phase1():
        for k in range(HG // 2):
            start(cp_g0(k))
        start(cp_xc(0))
        start(cp_xc(1))
        for k in range(len(SETS)):
            start(cp_set(k))
        start(cp_rest())
        zero_s[0] = 0
        kb_s[:, BR:BR + HALO, :] = jnp.zeros((8, HALO, 128), f32)
        vb_s[:, BR:BR + HALO, :] = jnp.zeros((8, HALO, 128), f32)
        for k in range(HG // 2):
            wait(cp_g0(k))
            convert_slice(0, 0, 2 * k)
            convert_slice(0, 0, 2 * k + 1)
        extract(0, 0, 0)
        wait(cp_xc(0))
        proj(0, 0, True)
        s_main, s_ext = qk(0, 0)
        proj(0, 1, True)
        softmax_pv(0, 0, s_main, s_ext, causal_tri(), vn)()
        wait(cp_xc(1))
        wait(cp_set(0))
        jax.lax.fori_loop(0, H, head_body, 0)
        wait(cp_rest())
        jax.lax.fori_loop(0, 8, bprep_wo, 0)

    @pl.when(step > 1)
    def _phase2():
        t = step - 2
        r0 = pl.multiple_of(t * BR, BR)
        never = zero_s[0] > 0
        ctx = jnp.concatenate([big[rows(h * S + r0, BR, BR), :] for h in range(H)], axis=1)
        nstage = (M // 128) * KS
        per = (BR // CH) // nstage
        kw = (H * D) // KS
        tok = None
        stage = 0
        half = []
        for p in range(M // 128):
            res = None
            for kk in range(KS):
                for cch in range(stage * per, (stage + 1) * per):
                    outs = b_attn_chunk(r0, cch, never, tok)
                    half.append(outs)
                    if len(half) * CH == 16:
                        a0 = (cch + 1) * CH - 16
                        for j in range(8):
                            ob_s[a0:a0 + 16, j * 128:(j + 1) * 128] = jnp.concatenate(
                                [hf[j] for hf in half], axis=0).astype(bf16)
                        half = []
                part = _dot(ctx[:, kk * kw:(kk + 1) * kw], wo_s[kk * kw:(kk + 1) * kw, p * 128:(p + 1) * 128])
                res = part if res is None else res + part
                tok = res[0:CH, :]
                stage += 1
            o_ref[:, p * 128:(p + 1) * 128] = res.astype(o_ref.dtype)
        wob = jnp.concatenate(
            [big[WOB_BASE + nc * M:WOB_BASE + (nc + 1) * M, :] for nc in range(8)], axis=1)
        o_ref[:, M:2 * M] = _dot(ob_s[...], wob).astype(o_ref.dtype)

    @pl.when(jnp.logical_and(step >= 1, step <= NB))
    def _phase2_qkv():
        b_qkv(step - 1)


@jax.jit
def pallas_concat_heads__compressed_kv_cla__sliding_local_dilated__prompt_kernel(
    A_x: jax.Array,
    A_c_kv: jax.Array,
    A_w_q: jax.Array,
    A_w_uk: jax.Array,
    A_w_uv: jax.Array,
    A_w_o: jax.Array,
    B_x: jax.Array,
    B_wqkv: jax.Array,
    B_wo: jax.Array,
):
    x = A_x.reshape(S, M)
    c = A_c_kv.reshape(S, DC)
    wo = A_w_o.reshape(H * D, M)
    xb = B_x.reshape(S, M)

    any_spec = pl.BlockSpec(memory_space=pl.ANY)
    V = pltpu.VMEM
    scratch = [
        V((S, M), bf16),
        V((S, DC), bf16),
        V((NG, M, HG, D), bf16),
        V((NG, DC, HG, D), bf16),
        V((NG, DC, HG, D), bf16),
        V((2, M * HG, D), f32),
        V((2, DC * HG, D), f32),
        V((2, DC * HG, D), f32),
        V((2, M + 2 * DC, D), bf16),
        V((S, D), bf16),
        V((S, D), bf16),
        V((2 * BQ, D), bf16),
        V((POOL_ROWS, D), bf16),
        V((H * D, M), bf16),
        V((S, M), bf16),
        V((M, 3 * M), bf16),
        V((M, M), bf16),
        V((8, 128, 128), f32),
        V((8, BR, 128), f32),
        V((8, BR + HALO, 128), f32),
        V((8, BR + HALO, 128), f32),
        V((BR, M), bf16),
        pltpu.SMEM((1,), jnp.int32),
        pltpu.SemaphoreType.DMA((13,)),
    ]
    out = pl.pallas_call(
        _kernel,
        grid=(2 + NB,),
        in_specs=[any_spec] * 9,
        out_specs=pl.BlockSpec((BR, 2 * M), lambda s: (jnp.maximum(s - 2, 0), 0)),
        out_shape=jax.ShapeDtypeStruct((S, 2 * M), bf16),
        scratch_shapes=scratch,
        compiler_params=pltpu.CompilerParams(
            dimension_semantics=("arbitrary",),
            vmem_limit_bytes=120 * 1024 * 1024,
            disable_bounds_checks=True,
        ),
        name="fused_mla_local",
    )(x, c, A_w_q, A_w_uk, A_w_uv, wo, xb, B_wqkv, B_wo)
    return out.reshape(1, S, 2 * M)
```

```python
import jax
import jax.numpy as jnp
import jax.experimental.pallas as pl
import jax.experimental.pallas.tpu as pltpu

bf16 = jnp.bfloat16
f32 = jnp.float32

S = 2048
H = 32
D = 128
M = 1024
DC = 512
HG = 8
NG = H // HG
BQ = 256
NQ = S // BQ
HB = 128
BW = 8
BDIL = 2
BH = 32
BDH = 32
HALO = 16
BR = 256
NB = S // BR
CH = 8
KS = 4
LOG2E = 1.4426950408889634
NEG = -1e30
NT = (((1,), (1,)), ((), ()))
NWQ = 24
WQ_CHUNKS = ((0, 1), (1, 3), (4, 4), (8, 4), (12, 4), (16, 4), (20, 4))
CONV_AT = 2
EXT_AT = 2


def _dot(a, b):
    return jnp.dot(a, b, preferred_element_type=f32)


def _dot_nt(a, b):
    return jax.lax.dot_general(a, b, NT, preferred_element_type=f32)


def _recip(x):
    r = pl.reciprocal(x, approx=True)
    return r * (2.0 - x * r)


def _kernel(x_hbm, c_hbm, wq_hbm, wuk_hbm, wuv_hbm, wo_hbm, xb_hbm, wqkv_hbm, wob_hbm,
            o_ref,
            x_s, c_s, rawq, rawk, rawv, tq, tk, tv,
            wbuf, ka, va, vn, big, wo_s, xb_s, wqkv_s, wob_s, wt_s, wobp_s,
            tb, qb_s, kb_s, vb_s, ob_s, zero_s, sems):
    step = pl.program_id(0)
    zz = step

    SEM_WQ, SEM_SET, SEM_LATE = 0, len(WQ_CHUNKS), len(WQ_CHUNKS) + NB
    MQ, MK = M // HG, DC // HG

    def cp_slices(g, s0, n, sem):
        heads = pl.ds(g * HG, HG)
        return [
            pltpu.make_async_copy(wuk_hbm.at[pl.ds(s0 * MK, n * MK), heads, :], rawk.at[g, pl.ds(s0 * MK, n * MK)], sem),
            pltpu.make_async_copy(wuv_hbm.at[pl.ds(s0 * MK, n * MK), heads, :], rawv.at[g, pl.ds(s0 * MK, n * MK)], sem),
            pltpu.make_async_copy(wq_hbm.at[pl.ds(s0 * MQ, n * MQ), heads, :], rawq.at[g, pl.ds(s0 * MQ, n * MQ)], sem),
        ]

    def cp_wq(k):
        t0, nt = WQ_CHUNKS[k]
        cols = pl.ds(t0 * 128, nt * 128)
        return [pltpu.make_async_copy(wqkv_hbm.at[:, cols], wqkv_s.at[:, cols], sems.at[SEM_WQ + k])]

    def cp_set(t):
        sem = sems.at[SEM_SET + t]
        r = pl.ds(t * BR, BR)
        f = pl.ds(t * 128, 128)
        return [pltpu.make_async_copy(xb_hbm.at[r], xb_s.at[r], sem),
                pltpu.make_async_copy(wob_hbm.at[f], wob_s.at[f], sem)] + cp_slices(0, t, 1, sem)

    def cp_late():
        sem = sems.at[SEM_LATE]
        cps = [pltpu.make_async_copy(c_hbm, c_s, sem), pltpu.make_async_copy(x_hbm, x_s, sem)]
        for g in range(1, NG):
            cps += cp_slices(g, 0, HG, sem)
        return cps + [pltpu.make_async_copy(wo_hbm, wo_s, sem)]

    def start(cps):
        for cp in cps:
            cp.start()

    def wait(cps):
        for cp in cps:
            cp.wait()

    def rows(start, size, align):
        return pl.ds(start if isinstance(start, int) else pl.multiple_of(start, align), size)

    def convert_slice(g, par, sl):
        mq = M // HG
        m0 = sl * mq if isinstance(sl, int) else pl.multiple_of(sl * mq, mq)
        tq[par, pl.ds(m0 * HG, mq * HG), :] = (
            rawq[g, pl.ds(m0, mq)].astype(f32).reshape(mq * HG, D))
        mk = DC // HG
        k0 = sl * mk if isinstance(sl, int) else pl.multiple_of(sl * mk, mk)
        tk[par, pl.ds(k0 * HG, mk * HG), :] = (
            rawk[g, pl.ds(k0, mk)].astype(f32).reshape(mk * HG, D))
        tv[par, pl.ds(k0 * HG, mk * HG), :] = (
            rawv[g, pl.ds(k0, mk)].astype(f32).reshape(mk * HG, D))

    def extract(par, j, wp):
        wbuf[wp, 0:M, :] = tq[par, pl.ds(j, M, stride=HG), :].astype(bf16)
        wbuf[wp, M:M + DC, :] = tk[par, pl.ds(j, DC, stride=HG), :].astype(bf16)
        wbuf[wp, M + DC:M + 2 * DC, :] = tv[par, pl.ds(j, DC, stride=HG), :].astype(bf16)

    def proj(h, i, staged):
        r = slice(i * BQ, (i + 1) * BQ)
        wp = h % 2
        q = _dot(x_s[r, :], wbuf[wp, 0:M, :])
        big[rows((h + zz) * S + i * BQ, BQ, BQ), :] = (q * (D ** -0.5 * LOG2E)).astype(bf16)
        wkv = jnp.concatenate([wbuf[wp, M:M + DC, :], wbuf[wp, M + DC:M + 2 * DC, :]], axis=1)
        kv = _dot(c_s[r, :], wkv)
        ka[r, :] = kv[:, :D].astype(bf16)
        if staged:
            vn[r, :] = kv[:, D:].astype(bf16)
        else:
            va[r, :] = kv[:, D:].astype(bf16)

    def qk(h, i):
        r0 = i * BQ
        q = big[rows((h + zz) * S + r0, BQ, BQ), :]
        s_main = _dot_nt(q, ka[0:r0 + HB, :])
        q_lo = big[rows((h + zz) * S + r0 + HB, HB, HB), :]
        s_ext = _dot_nt(q_lo, ka[r0 + HB:r0 + BQ, :])
        return s_main, s_ext

    def softmax_pv(h, i, s_main, s_ext, tri, vr):
        r0 = i * BQ
        nt = 2 * i + 1
        tiles = [s_main[:, t * HB:(t + 1) * HB] for t in range(nt)]
        last = tiles[-1]
        tiles[-1] = jnp.concatenate([jnp.where(tri, last[:HB], NEG), last[HB:]], axis=0)
        ext = jnp.where(tri, s_ext, NEG)
        mt = tiles[0]
        for t in range(1, nt):
            mt = jnp.maximum(mt, tiles[t])
        mt = jnp.concatenate([mt[:HB], jnp.maximum(mt[HB:], ext)], axis=0)
        m = jnp.max(mt, axis=1, keepdims=True)
        pe = jnp.exp2(ext - m[HB:])
        ps = [jnp.exp2(tiles[t] - m) for t in range(nt)]
        p_main = jnp.concatenate(ps, axis=1).astype(bf16)
        lt = ps[0]
        for p in ps[1:]:
            lt = lt + p
        cm = _dot(p_main, vr[0:r0 + HB, :])
        lt = jnp.concatenate([lt[:HB], lt[HB:] + pe], axis=0)
        l = jnp.sum(lt, axis=1, keepdims=True)
        ce = _dot(pe.astype(bf16), vr[r0 + HB:r0 + BQ, :])
        cm = jnp.concatenate([cm[:HB], cm[HB:] + ce], axis=0)
        val = (cm * _recip(l)).astype(bf16)

        def store():
            big[rows(h * S + r0, BQ, BQ), :] = val
        return store

    def causal_tri():
        row = jax.lax.broadcasted_iota(jnp.int32, (HB, HB), 0)
        col = jax.lax.broadcasted_iota(jnp.int32, (HB, HB), 1)
        return col <= row

    def head_body(h, carry):
        hn = h + 1
        tri = causal_tri()
        va[0:2 * BQ, :] = vn[...]
        seq = [(h, i, va) for i in range(1, NQ)] + [(hn, 0, vn)]
        pend = []
        for hh, i, vr in seq:
            s_main, s_ext = qk(hh, i)
            if hh is hn:
                proj(hn, 1, True)
            elif i + 1 == NQ:
                proj(hn, 0, True)
            else:
                proj(h, i + 1, False)
            if hh is h and i == CONV_AT:
                gc = h // HG + 1
                convert_slice(jnp.minimum(gc, NG - 1), gc % 2, h % HG)
            if hh is h and i == EXT_AT:
                he = jnp.minimum(hn, H - 1)
                extract((he // HG) % 2, he % HG, hn % 2)
            while len(pend) >= 2:
                pend.pop(0)()
            pend.append(softmax_pv(hh, i, s_main, s_ext, tri, vr))
        for st in pend:
            st()
        return carry

    def permute_rows(blk, mc):
        for h4 in range(4):
            tb[mc, pl.ds(h4, 32, stride=4), :] = blk[h4 * 32:(h4 + 1) * 32, :]

    def bprep_qkv(t, carry):
        for k in range(1, len(WQ_CHUNKS)):
            @pl.when(t == WQ_CHUNKS[k][0])
            def _():
                wait(cp_wq(k))
        part = t // 8
        g = t % 8
        for mc in range(M // 128):
            permute_rows(
                wqkv_s[mc * 128:(mc + 1) * 128, pl.ds(pl.multiple_of(t * 128, 128), 128)].astype(f32).T, mc)
        for mc in range(M // 128):
            for i in range(8):
                wt_s[mc, rows(part * M + i * 128 + g * 16, 16, 16), :] = (
                    tb[mc, i * 16:(i + 1) * 16, :].astype(bf16))
        return carry

    def bprep_wo(g):
        for nc in range(M // 128):
            permute_rows(wob_s[rows(g * 128, 128, 128), nc * 128:(nc + 1) * 128].astype(f32), nc)
        for nc in range(M // 128):
            for i in range(8):
                wobp_s[nc, rows(i * 128 + g * 16, 16, 16), :] = tb[nc, i * 16:(i + 1) * 16, :].astype(bf16)

    def b_qkv(t, carry):
        wait(cp_set(t))
        wt = jnp.concatenate([wt_s[mc] for mc in range(8)], axis=1)
        qkv = _dot_nt(xb_s[rows(t * BR, BR, BR), :], wt)
        rq = rows(t * BR, BR, BR)
        rk = rows(t * BR + HALO, BR, HALO)
        for j in range(8):
            qb_s[j, rq, :] = qkv[:, j * 128:(j + 1) * 128] * (BDH ** -0.5 * LOG2E)
            kb_s[j, rk, :] = qkv[:, 1024 + j * 128:1024 + (j + 1) * 128]
            vb_s[j, rk, :] = qkv[:, 2048 + j * 128:2048 + (j + 1) * 128]
        convert_slice(0, 0, t)
        bprep_wo(t)
        return carry

    def b_attn_chunk(r0, cch, never, tok):
        a0 = cch * CH
        lane = jax.lax.broadcasted_iota(jnp.int32, (CH, 128), 1)
        b2 = (lane & 4) != 0
        b3 = (lane & 8) != 0
        qs = [qb_s[j, pl.ds(r0 + a0, CH), :] for j in range(8)]
        if tok is not None:
            qs = [jnp.where(never, tok, q) for q in qs]
        logit = []
        for w in range(BW):
            acc = None
            for j in range(8):
                term = qs[j] * kb_s[j, pl.ds(r0 + (HALO + a0 - BDIL * w), CH), :]
                acc = term if acc is None else acc + term
            acc = acc + jnp.where(b2, pltpu.roll(acc, 4, 1), pltpu.roll(acc, 124, 1))
            acc = acc + jnp.where(b3, pltpu.roll(acc, 8, 1), pltpu.roll(acc, 120, 1))
            if a0 < BDIL * w:
                pos = jax.lax.broadcasted_iota(jnp.int32, (CH, 128), 0) + (r0 + a0)
                acc = jnp.where(pos >= BDIL * w, acc, NEG)
            logit.append(acc)
        mx = logit[0]
        for w in range(1, BW):
            mx = jnp.maximum(mx, logit[w])
        e = [jnp.exp2(lg - mx) for lg in logit]
        den = e[0]
        for w in range(1, BW):
            den = den + e[w]
        inv = _recip(den)
        e = [ew * inv for ew in e]
        outs = []
        for j in range(8):
            acc = None
            for w in range(BW):
                term = e[w] * vb_s[j, pl.ds(r0 + (HALO + a0 - BDIL * w), CH), :]
                acc = term if acc is None else acc + term
            outs.append(acc)
        return outs

    @pl.when(step == 0)
    def _phase1():
        for k in range(len(WQ_CHUNKS)):
            start(cp_wq(k))
        for t in range(NB):
            start(cp_set(t))
        start(cp_late())
        zero_s[0] = 0
        kb_s[:, 0:HALO, :] = jnp.zeros((8, HALO, 128), f32)
        vb_s[:, 0:HALO, :] = jnp.zeros((8, HALO, 128), f32)
        wait(cp_wq(0))
        jax.lax.fori_loop(0, NWQ, bprep_qkv, 0)
        jax.lax.fori_loop(0, NB, b_qkv, 0)
        wait(cp_late())
        extract(0, 0, 0)
        proj(0, 0, True)
        s_main, s_ext = qk(0, 0)
        proj(0, 1, True)
        softmax_pv(0, 0, s_main, s_ext, causal_tri(), vn)()
        jax.lax.fori_loop(0, H, head_body, 0)

    @pl.when(step > 0)
    def _phase2():
        t = step - 1
        r0 = pl.multiple_of(t * BR, BR)
        never = zero_s[0] > 0
        ctx = jnp.concatenate([big[rows(h * S + r0, BR, BR), :] for h in range(H)], axis=1)
        nstage = (M // 128) * KS
        per = (BR // CH) // nstage
        kw = (H * D) // KS
        tok = None
        stage = 0
        half = []
        for p in range(M // 128):
            res = None
            for kk in range(KS):
                for cch in range(stage * per, (stage + 1) * per):
                    outs = b_attn_chunk(r0, cch, never, tok)
                    half.append(outs)
                    if len(half) * CH == 16:
                        a0 = (cch + 1) * CH - 16
                        for j in range(8):
                            ob_s[a0:a0 + 16, j * 128:(j + 1) * 128] = jnp.concatenate(
                                [hf[j] for hf in half], axis=0).astype(bf16)
                        half = []
                part = _dot(ctx[:, kk * kw:(kk + 1) * kw], wo_s[kk * kw:(kk + 1) * kw, p * 128:(p + 1) * 128])
                res = part if res is None else res + part
                tok = res[0:CH, :]
                stage += 1
            o_ref[:, p * 128:(p + 1) * 128] = res.astype(o_ref.dtype)
        wob = jnp.concatenate([wobp_s[nc] for nc in range(8)], axis=1)
        o_ref[:, M:2 * M] = _dot(ob_s[...], wob).astype(o_ref.dtype)


@jax.jit
def pallas_concat_heads__compressed_kv_cla__sliding_local_dilated__prompt_kernel(
    A_x: jax.Array,
    A_c_kv: jax.Array,
    A_w_q: jax.Array,
    A_w_uk: jax.Array,
    A_w_uv: jax.Array,
    A_w_o: jax.Array,
    B_x: jax.Array,
    B_wqkv: jax.Array,
    B_wo: jax.Array,
):
    x = A_x.reshape(S, M)
    c = A_c_kv.reshape(S, DC)
    wo = A_w_o.reshape(H * D, M)
    xb = B_x.reshape(S, M)

    any_spec = pl.BlockSpec(memory_space=pl.ANY)
    V = pltpu.VMEM
    scratch = [
        V((S, M), bf16),
        V((S, DC), bf16),
        V((NG, M, HG, D), bf16),
        V((NG, DC, HG, D), bf16),
        V((NG, DC, HG, D), bf16),
        V((2, M * HG, D), f32),
        V((2, DC * HG, D), f32),
        V((2, DC * HG, D), f32),
        V((2, M + 2 * DC, D), bf16),
        V((S, D), bf16),
        V((S, D), bf16),
        V((2 * BQ, D), bf16),
        V(((H + 1) * S, D), bf16),
        V((H * D, M), bf16),
        V((S, M), bf16),
        V((M, 3 * M), bf16),
        V((M, M), bf16),
        V((8, 3 * M, 128), bf16),
        V((8, M, 128), bf16),
        V((8, 128, 128), f32),
        V((8, S, 128), f32),
        V((8, S + HALO, 128), f32),
        V((8, S + HALO, 128), f32),
        V((BR, M), bf16),
        pltpu.SMEM((1,), jnp.int32),
        pltpu.SemaphoreType.DMA((len(WQ_CHUNKS) + NB + 1,)),
    ]
    out = pl.pallas_call(
        _kernel,
        grid=(1 + NB,),
        in_specs=[any_spec] * 9,
        out_specs=pl.BlockSpec((BR, 2 * M), lambda s: (jnp.maximum(s - 1, 0), 0)),
        out_shape=jax.ShapeDtypeStruct((S, 2 * M), bf16),
        scratch_shapes=scratch,
        compiler_params=pltpu.CompilerParams(
            dimension_semantics=("arbitrary",),
            vmem_limit_bytes=124 * 1024 * 1024,
            disable_bounds_checks=True,
        ),
        name="fused_mla_local",
    )(x, c, A_w_q, A_w_uk, A_w_uv, wo, xb, B_wqkv, B_wo)
    return out.reshape(1, S, 2 * M)
```

```python
import jax
import jax.numpy as jnp
import jax.experimental.pallas as pl
import jax.experimental.pallas.tpu as pltpu

bf16 = jnp.bfloat16
f32 = jnp.float32

S = 2048
H = 32
D = 128
M = 1024
DC = 512
HG = 8
NG = H // HG
BQ = 256
NQ = S // BQ
HB = 128
BW = 8
BDIL = 2
BH = 32
BDH = 32
HALO = 16
BR = 256
NB = S // BR
CH = 8
KS = 4
LOG2E = 1.4426950408889634
NEG = -1e30
NT = (((1,), (1,)), ((), ()))
NWQ = 24
WQ_CHUNKS = ((0, 1), (1, 3), (4, 4))
PR = 512
NPR = S // PR
CONV_AT = 2
EXT_AT = 2
LAG = 2
KV_FIRST = False


def _dot(a, b):
    return jnp.dot(a, b, preferred_element_type=f32)


def _dot_nt(a, b):
    return jax.lax.dot_general(a, b, NT, preferred_element_type=f32)


def _recip(x):
    r = pl.reciprocal(x, approx=True)
    return r * (2.0 - x * r)


def _kernel(x_hbm, c_hbm, wq_hbm, wuk_hbm, wuv_hbm, wo_hbm, xb_hbm, wqkv_hbm, wob_hbm,
            o_ref,
            x_s, c_s, rawq, rawk, rawv, tq, tk, tv,
            wbuf, ka, va, vn, big, wo_s, xb_s, wqkv_s, wob_s, wt_s, wobp_s,
            tb, qkv_s, ob_s, zero_s, sems):
    step = pl.program_id(0)
    zz = step

    SEM_WQ, SEM_SET, SEM_LATE = 0, len(WQ_CHUNKS), len(WQ_CHUNKS) + 2 * NPR
    MQ, MK = M // HG, DC // HG

    def cp_slices(g, s0, n, sem):
        heads = pl.ds(g * HG, HG)
        return [
            pltpu.make_async_copy(wuk_hbm.at[pl.ds(s0 * MK, n * MK), heads, :], rawk.at[g, pl.ds(s0 * MK, n * MK)], sem),
            pltpu.make_async_copy(wuv_hbm.at[pl.ds(s0 * MK, n * MK), heads, :], rawv.at[g, pl.ds(s0 * MK, n * MK)], sem),
            pltpu.make_async_copy(wq_hbm.at[pl.ds(s0 * MQ, n * MQ), heads, :], rawq.at[g, pl.ds(s0 * MQ, n * MQ)], sem),
        ]

    def cp_wq(k):
        t0, nt = WQ_CHUNKS[k]
        cols = pl.ds(t0 * 128, nt * 128)
        return [pltpu.make_async_copy(wqkv_hbm.at[:, cols], wqkv_s.at[:, cols], sems.at[SEM_WQ + k])]

    def cp_set(it):
        sem = sems.at[SEM_SET + it]
        cols = pl.ds((8 + 2 * it) * 128, 256)
        cps = [pltpu.make_async_copy(wqkv_hbm.at[:, cols], wqkv_s.at[:, cols], sem)]
        if it < NPR:
            r = pl.ds(it * PR, PR)
            cps.insert(0, pltpu.make_async_copy(xb_hbm.at[r], xb_s.at[r], sem))
        return cps

    def cp_late():
        sem = sems.at[SEM_LATE]
        cps = [pltpu.make_async_copy(c_hbm, c_s, sem), pltpu.make_async_copy(x_hbm, x_s, sem)]
        for g in range(1, NG):
            cps += cp_slices(g, 0, HG, sem)
        return cps + [pltpu.make_async_copy(wo_hbm, wo_s, sem)]

    def cp_mid():
        sem = sems.at[SEM_LATE + 1]
        return cp_slices(0, 0, HG, sem) + [pltpu.make_async_copy(wob_hbm, wob_s, sem)]

    def start(cps):
        for cp in cps:
            cp.start()

    def wait(cps):
        for cp in cps:
            cp.wait()

    def rows(start, size, align):
        return pl.ds(start if isinstance(start, int) else pl.multiple_of(start, align), size)

    def convert_slice(g, par, sl):
        mq = M // HG
        m0 = sl * mq if isinstance(sl, int) else pl.multiple_of(sl * mq, mq)
        tq[par, pl.ds(m0 * HG, mq * HG), :] = (
            rawq[g, pl.ds(m0, mq)].astype(f32).reshape(mq * HG, D))
        mk = DC // HG
        k0 = sl * mk if isinstance(sl, int) else pl.multiple_of(sl * mk, mk)
        tk[par, pl.ds(k0 * HG, mk * HG), :] = (
            rawk[g, pl.ds(k0, mk)].astype(f32).reshape(mk * HG, D))
        tv[par, pl.ds(k0 * HG, mk * HG), :] = (
            rawv[g, pl.ds(k0, mk)].astype(f32).reshape(mk * HG, D))

    def extract(par, j, wp):
        wbuf[wp, 0:M, :] = tq[par, pl.ds(j, M, stride=HG), :].astype(bf16)
        wbuf[wp, M:M + DC, :] = tk[par, pl.ds(j, DC, stride=HG), :].astype(bf16)
        wbuf[wp, M + DC:M + 2 * DC, :] = tv[par, pl.ds(j, DC, stride=HG), :].astype(bf16)

    def proj(h, i, staged):
        r = slice(i * BQ, (i + 1) * BQ)
        wp = h % 2

        def q_part():
            q = _dot(x_s[r, :], wbuf[wp, 0:M, :])
            big[rows((h + zz) * S + i * BQ, BQ, BQ), :] = (q * (D ** -0.5 * LOG2E)).astype(bf16)

        def kv_part():
            wkv = jnp.concatenate([wbuf[wp, M:M + DC, :], wbuf[wp, M + DC:M + 2 * DC, :]], axis=1)
            kv = _dot(c_s[r, :], wkv)
            ka[r, :] = kv[:, :D].astype(bf16)
            if staged:
                vn[r, :] = kv[:, D:].astype(bf16)
            else:
                va[r, :] = kv[:, D:].astype(bf16)

        if KV_FIRST:
            kv_part()
            q_part()
        else:
            q_part()
            kv_part()

    def qk(h, i):
        r0 = i * BQ
        q = big[rows((h + zz) * S + r0, BQ, BQ), :]
        s_main = _dot_nt(q, ka[0:r0 + HB, :])
        q_lo = big[rows((h + zz) * S + r0 + HB, HB, HB), :]
        s_ext = _dot_nt(q_lo, ka[r0 + HB:r0 + BQ, :])
        return s_main, s_ext

    def softmax_pv(h, i, s_main, s_ext, tri, vr):
        r0 = i * BQ
        nt = 2 * i + 1
        tiles = [s_main[:, t * HB:(t + 1) * HB] for t in range(nt)]
        last = tiles[-1]
        tiles[-1] = jnp.concatenate([jnp.where(tri, last[:HB], NEG), last[HB:]], axis=0)
        ext = jnp.where(tri, s_ext, NEG)
        mt = tiles[0]
        for t in range(1, nt):
            mt = jnp.maximum(mt, tiles[t])
        mt = jnp.concatenate([mt[:HB], jnp.maximum(mt[HB:], ext)], axis=0)
        m = jnp.max(mt, axis=1, keepdims=True)
        pe = jnp.exp2(ext - m[HB:])
        ps = [jnp.exp2(tiles[t] - m) for t in range(nt)]
        p_main = jnp.concatenate(ps, axis=1).astype(bf16)
        lt = ps[0]
        for p in ps[1:]:
            lt = lt + p
        cm = _dot(p_main, vr[0:r0 + HB, :])
        lt = jnp.concatenate([lt[:HB], lt[HB:] + pe], axis=0)
        l = jnp.sum(lt, axis=1, keepdims=True)
        ce = _dot(pe.astype(bf16), vr[r0 + HB:r0 + BQ, :])
        cm = jnp.concatenate([cm[:HB], cm[HB:] + ce], axis=0)
        val = (cm * _recip(l)).astype(bf16)

        def store():
            big[rows(h * S + r0, BQ, BQ), :] = val
        return store

    def causal_tri():
        row = jax.lax.broadcasted_iota(jnp.int32, (HB, HB), 0)
        col = jax.lax.broadcasted_iota(jnp.int32, (HB, HB), 1)
        return col <= row

    def head_body(h, carry):
        hn = h + 1
        tri = causal_tri()
        va[0:2 * BQ, :] = vn[...]
        seq = [(h, i, va) for i in range(1, NQ)] + [(hn, 0, vn)]
        pend = []
        for hh, i, vr in seq:
            s_main, s_ext = qk(hh, i)
            if hh is hn:
                proj(hn, 1, True)
            elif i + 1 == NQ:
                proj(hn, 0, True)
            else:
                proj(h, i + 1, False)
            if hh is h and i == CONV_AT:
                gc = h // HG + 1
                convert_slice(jnp.minimum(gc, NG - 1), gc % 2, h % HG)
            if hh is h and i == EXT_AT:
                he = jnp.minimum(hn, H - 1)
                extract((he // HG) % 2, he % HG, hn % 2)
            while len(pend) >= LAG:
                pend.pop(0)()
            pend.append(softmax_pv(hh, i, s_main, s_ext, tri, vr))
        for st in pend:
            st()
        return carry

    def permute_rows(blk, slot, mc):
        for h4 in range(4):
            tb[slot, mc, pl.ds(h4, 32, stride=4), :] = blk[h4 * 32:(h4 + 1) * 32, :]

    def bprep_qkv(t, slot):
        part = t // 8
        g = t % 8
        for mc in range(M // 128):
            permute_rows(
                wqkv_s[mc * 128:(mc + 1) * 128, pl.ds(pl.multiple_of(t * 128, 128), 128)].astype(f32).T, slot, mc)
        for mc in range(M // 128):
            for i in range(8):
                wt_s[mc, rows(part * M + i * 128 + g * 16, 16, 16), :] = (
                    tb[slot, mc, i * 16:(i + 1) * 16, :].astype(bf16))

    def bprep_q_part(t, carry):
        for k in range(1, len(WQ_CHUNKS)):
            @pl.when(t == WQ_CHUNKS[k][0])
            def _():
                wait(cp_wq(k))
        bprep_qkv(t, 0)
        return carry

    def bprep_wo(g, slot):
        for nc in range(M // 128):
            permute_rows(wob_s[rows(g * 128, 128, 128), nc * 128:(nc + 1) * 128].astype(f32), slot, nc)
        for nc in range(M // 128):
            for i in range(8):
                wobp_s[nc, rows(i * 128 + g * 16, 16, 16), :] = tb[slot, nc, i * 16:(i + 1) * 16, :].astype(bf16)

    def b_proj(part, u):
        wt = jnp.concatenate([wt_s[mc, rows(part * M, M, M), :] for mc in range(8)], axis=1)
        res = _dot_nt(xb_s[rows(u * PR, PR, PR), :], wt)
        if not isinstance(part, int):
            res = res * jnp.where(part == 0, BDH ** -0.5 * LOG2E, 1.0)
        rr = rows(u * PR + HALO, PR, HALO)
        for j in range(8):
            qkv_s[part, j, rr, :] = res[:, j * 128:(j + 1) * 128]

    def b_proj_qk(it, carry):
        for k in range(2 * NPR):
            @pl.when(it == k)
            def _():
                wait(cp_set(k))
        b_proj(it // NPR, it % NPR)
        bprep_qkv(8 + 2 * it, 0)
        bprep_qkv(9 + 2 * it, 1)
        return carry

    def b_proj_v(u, carry):
        b_proj(2, u)
        for k in range(2):
            convert_slice(0, 0, 2 * u + k)
            bprep_wo(2 * u + k, k)
        return carry

    def b_attn_chunk(r0, cch, never, tok):
        a0 = cch * CH
        lane = jax.lax.broadcasted_iota(jnp.int32, (CH, 128), 1)
        b2 = (lane & 4) != 0
        b3 = (lane & 8) != 0
        qs = [qkv_s[0, j, pl.ds(r0 + (HALO + a0), CH), :] for j in range(8)]
        if tok is not None:
            qs = [jnp.where(never, tok, q) for q in qs]
        logit = []
        for w in range(BW):
            acc = None
            for j in range(8):
                term = qs[j] * qkv_s[1, j, pl.ds(r0 + (HALO + a0 - BDIL * w), CH), :]
                acc = term if acc is None else acc + term
            acc = acc + jnp.where(b2, pltpu.roll(acc, 4, 1), pltpu.roll(acc, 124, 1))
            acc = acc + jnp.where(b3, pltpu.roll(acc, 8, 1), pltpu.roll(acc, 120, 1))
            if a0 < BDIL * w:
                pos = jax.lax.broadcasted_iota(jnp.int32, (CH, 128), 0) + (r0 + a0)
                acc = jnp.where(pos >= BDIL * w, acc, NEG)
            logit.append(acc)
        mx = logit[0]
        for w in range(1, BW):
            mx = jnp.maximum(mx, logit[w])
        e = [jnp.exp2(lg - mx) for lg in logit]
        den = e[0]
        for w in range(1, BW):
            den = den + e[w]
        inv = _recip(den)
        e = [ew * inv for ew in e]
        outs = []
        for j in range(8):
            acc = None
            for w in range(BW):
                term = e[w] * qkv_s[2, j, pl.ds(r0 + (HALO + a0 - BDIL * w), CH), :]
                acc = term if acc is None else acc + term
            outs.append(acc)
        return outs

    @pl.when(step == 0)
    def _phase1():
        for k in range(len(WQ_CHUNKS)):
            start(cp_wq(k))
        for it in range(2 * NPR):
            start(cp_set(it))
        start(cp_mid())
        start(cp_late())
        zero_s[0] = 0
        for part in range(1, 3):
            qkv_s[part, :, 0:HALO, :] = jnp.zeros((8, HALO, 128), f32)
        wait(cp_wq(0))
        jax.lax.fori_loop(0, 8, bprep_q_part, 0)
        jax.lax.fori_loop(0, 2 * NPR, b_proj_qk, 0)
        wait(cp_mid())
        jax.lax.fori_loop(0, NPR, b_proj_v, 0)
        wait(cp_late())
        extract(0, 0, 0)
        proj(0, 0, True)
        s_main, s_ext = qk(0, 0)
        proj(0, 1, True)
        softmax_pv(0, 0, s_main, s_ext, causal_tri(), vn)()
        jax.lax.fori_loop(0, H, head_body, 0)

    @pl.when(step > 0)
    def _phase2():
        t = step - 1
        r0 = pl.multiple_of(t * BR, BR)
        never = zero_s[0] > 0
        ctx = jnp.concatenate([big[rows(h * S + r0, BR, BR), :] for h in range(H)], axis=1)
        nstage = (M // 128) * KS
        per = (BR // CH) // nstage
        kw = (H * D) // KS
        tok = None
        stage = 0
        half = []
        for p in range(M // 128):
            res = None
            for kk in range(KS):
                for cch in range(stage * per, (stage + 1) * per):
                    outs = b_attn_chunk(r0, cch, never, tok)
                    half.append(outs)
                    if len(half) * CH == 16:
                        a0 = (cch + 1) * CH - 16
                        for j in range(8):
                            ob_s[a0:a0 + 16, j * 128:(j + 1) * 128] = jnp.concatenate(
                                [hf[j] for hf in half], axis=0).astype(bf16)
                        half = []
                part = _dot(ctx[:, kk * kw:(kk + 1) * kw], wo_s[kk * kw:(kk + 1) * kw, p * 128:(p + 1) * 128])
                res = part if res is None else res + part
                tok = res[0:CH, :]
                stage += 1
            o_ref[:, p * 128:(p + 1) * 128] = res.astype(o_ref.dtype)
        wob = jnp.concatenate([wobp_s[nc] for nc in range(8)], axis=1)
        o_ref[:, M:2 * M] = _dot(ob_s[...], wob).astype(o_ref.dtype)


@jax.jit
def pallas_concat_heads__compressed_kv_cla__sliding_local_dilated__prompt_kernel(
    A_x: jax.Array,
    A_c_kv: jax.Array,
    A_w_q: jax.Array,
    A_w_uk: jax.Array,
    A_w_uv: jax.Array,
    A_w_o: jax.Array,
    B_x: jax.Array,
    B_wqkv: jax.Array,
    B_wo: jax.Array,
):
    x = A_x.reshape(S, M)
    c = A_c_kv.reshape(S, DC)
    wo = A_w_o.reshape(H * D, M)
    xb = B_x.reshape(S, M)

    any_spec = pl.BlockSpec(memory_space=pl.ANY)
    V = pltpu.VMEM
    scratch = [
        V((S, M), bf16),
        V((S, DC), bf16),
        V((NG, M, HG, D), bf16),
        V((NG, DC, HG, D), bf16),
        V((NG, DC, HG, D), bf16),
        V((2, M * HG, D), f32),
        V((2, DC * HG, D), f32),
        V((2, DC * HG, D), f32),
        V((2, M + 2 * DC, D), bf16),
        V((S, D), bf16),
        V((S, D), bf16),
        V((2 * BQ, D), bf16),
        V(((H + 1) * S, D), bf16),
        V((H * D, M), bf16),
        V((S, M), bf16),
        V((M, 3 * M), bf16),
        V((M, M), bf16),
        V((8, 3 * M, 128), bf16),
        V((8, M, 128), bf16),
        V((2, 8, 128, 128), f32),
        V((3, 8, S + HALO, 128), f32),
        V((BR, M), bf16),
        pltpu.SMEM((1,), jnp.int32),
        pltpu.SemaphoreType.DMA((len(WQ_CHUNKS) + 2 * NPR + 2,)),
    ]
    out = pl.pallas_call(
        _kernel,
        grid=(1 + NB,),
        in_specs=[any_spec] * 9,
        out_specs=pl.BlockSpec((BR, 2 * M), lambda s: (jnp.maximum(s - 1, 0), 0)),
        out_shape=jax.ShapeDtypeStruct((S, 2 * M), bf16),
        scratch_shapes=scratch,
        compiler_params=pltpu.CompilerParams(
            dimension_semantics=("arbitrary",),
            vmem_limit_bytes=124 * 1024 * 1024,
            disable_bounds_checks=True,
        ),
        name="fused_mla_local",
    )(x, c, A_w_q, A_w_uk, A_w_uv, wo, xb, B_wqkv, B_wo)
    return out.reshape(1, S, 2 * M)
```

```python
import jax
import jax.numpy as jnp
import jax.experimental.pallas as pl
import jax.experimental.pallas.tpu as pltpu

bf16 = jnp.bfloat16
f32 = jnp.float32

S = 2048
H = 32
D = 128
M = 1024
DC = 512
HG = 8
NG = H // HG
BQ = 256
NQ = S // BQ
HB = 128
BW = 8
BDIL = 2
BH = 32
BDH = 32
HALO = 16
BR = 256
NB = S // BR
CH = 8
KS = 4
LOG2E = 1.4426950408889634
NEG = -1e30
NT = (((1,), (1,)), ((), ()))
NWQ = 24
WQ_CHUNKS = ((0, 1), (1, 3), (4, 4))
PR = 512
NPR = S // PR
CONV_AT = 2
EXT_AT = 2
LAG = 2
KV_FIRST = False


def _dot(a, b):
    return jnp.dot(a, b, preferred_element_type=f32)


def _dot_nt(a, b):
    return jax.lax.dot_general(a, b, NT, preferred_element_type=f32)


def _recip(x):
    r = pl.reciprocal(x, approx=True)
    return r * (2.0 - x * r)


def _kernel(x_hbm, c_hbm, wq_hbm, wuk_hbm, wuv_hbm, wo_hbm, xb_hbm, wqkv_hbm, wob_hbm,
            o_ref,
            x_s, c_s, rawq, rawk, rawv, tq, tk, tv,
            wbuf, ka, va, vn, big, wo_s, xb_s, wqkv_s, wob_s, wt_s, wobp_s,
            tb, qkv_s, ob_s, zero_s, sems):
    step = pl.program_id(0)
    zz = step

    SEM_WQ, SEM_SET, SEM_LATE = 0, len(WQ_CHUNKS), len(WQ_CHUNKS) + 2 * NPR
    MQ, MK = M // HG, DC // HG

    def cp_slices(g, s0, n, sem):
        heads = pl.ds(g * HG, HG)
        return [
            pltpu.make_async_copy(wuk_hbm.at[pl.ds(s0 * MK, n * MK), heads, :], rawk.at[g, pl.ds(s0 * MK, n * MK)], sem),
            pltpu.make_async_copy(wuv_hbm.at[pl.ds(s0 * MK, n * MK), heads, :], rawv.at[g, pl.ds(s0 * MK, n * MK)], sem),
            pltpu.make_async_copy(wq_hbm.at[pl.ds(s0 * MQ, n * MQ), heads, :], rawq.at[g, pl.ds(s0 * MQ, n * MQ)], sem),
        ]

    def cp_wq(k):
        t0, nt = WQ_CHUNKS[k]
        cols = pl.ds(t0 * 128, nt * 128)
        return [pltpu.make_async_copy(wqkv_hbm.at[:, cols], wqkv_s.at[:, cols], sems.at[SEM_WQ + k])]

    def cp_set(it):
        sem = sems.at[SEM_SET + it]
        cols = pl.ds((8 + 2 * it) * 128, 256)
        cps = [pltpu.make_async_copy(wqkv_hbm.at[:, cols], wqkv_s.at[:, cols], sem)]
        if it < NPR:
            r = pl.ds(it * PR, PR)
            cps.insert(0, pltpu.make_async_copy(xb_hbm.at[r], xb_s.at[r], sem))
        return cps

    def cp_late():
        sem = sems.at[SEM_LATE]
        cps = [pltpu.make_async_copy(c_hbm, c_s, sem), pltpu.make_async_copy(x_hbm, x_s, sem)]
        for g in range(1, NG):
            cps += cp_slices(g, 0, HG, sem)
        return cps + [pltpu.make_async_copy(wo_hbm, wo_s, sem)]

    def cp_mid():
        sem = sems.at[SEM_LATE + 1]
        return cp_slices(0, 0, HG, sem) + [pltpu.make_async_copy(wob_hbm, wob_s, sem)]

    def start(cps):
        for cp in cps:
            cp.start()

    def wait(cps):
        for cp in cps:
            cp.wait()

    def rows(start, size, align):
        return pl.ds(start if isinstance(start, int) else pl.multiple_of(start, align), size)

    def convert_slice(g, par, sl):
        for raw, dst, n in ((rawq, tq, M // HG), (rawk, tk, DC // HG), (rawv, tv, DC // HG)):
            m0 = sl * n if isinstance(sl, int) else pl.multiple_of(sl * n, n)
            dst[par, pl.ds(m0 * 4, n * 4), :] = pltpu.bitcast(
                raw[g, pl.ds(m0, n)].reshape(n * HG, D), jnp.uint32)

    def extract(par, j, wp):
        shift = jnp.where(j % 2 == 0, 16, 0).astype(jnp.uint32)
        for src, r0, n in ((tq, 0, M), (tk, M, DC), (tv, M + DC, DC)):
            w = src[par, pl.ds(j // 2, n, stride=4), :]
            w = (w << shift) & jnp.uint32(0xFFFF0000)
            wbuf[wp, r0:r0 + n, :] = pltpu.bitcast(w, f32).astype(bf16)

    def proj(h, i, staged):
        r = slice(i * BQ, (i + 1) * BQ)
        wp = h % 2

        def q_part():
            q = _dot(x_s[r, :], wbuf[wp, 0:M, :])
            big[rows((h + zz) * S + i * BQ, BQ, BQ), :] = (q * (D ** -0.5 * LOG2E)).astype(bf16)

        def kv_part():
            wkv = jnp.concatenate([wbuf[wp, M:M + DC, :], wbuf[wp, M + DC:M + 2 * DC, :]], axis=1)
            kv = _dot(c_s[r, :], wkv)
            ka[r, :] = kv[:, :D].astype(bf16)
            if staged:
                vn[r, :] = kv[:, D:].astype(bf16)
            else:
                va[r, :] = kv[:, D:].astype(bf16)

        if KV_FIRST:
            kv_part()
            q_part()
        else:
            q_part()
            kv_part()

    def qk(h, i):
        r0 = i * BQ
        q = big[rows((h + zz) * S + r0, BQ, BQ), :]
        s_main = _dot_nt(q, ka[0:r0 + HB, :])
        q_lo = big[rows((h + zz) * S + r0 + HB, HB, HB), :]
        s_ext = _dot_nt(q_lo, ka[r0 + HB:r0 + BQ, :])
        return s_main, s_ext

    def softmax_pv(h, i, s_main, s_ext, tri, vr):
        r0 = i * BQ
        nt = 2 * i + 1
        tiles = [s_main[:, t * HB:(t + 1) * HB] for t in range(nt)]
        last = tiles[-1]
        tiles[-1] = jnp.concatenate([jnp.where(tri, last[:HB], NEG), last[HB:]], axis=0)
        ext = jnp.where(tri, s_ext, NEG)
        mt = tiles[0]
        for t in range(1, nt):
            mt = jnp.maximum(mt, tiles[t])
        mt = jnp.concatenate([mt[:HB], jnp.maximum(mt[HB:], ext)], axis=0)
        m = jnp.max(mt, axis=1, keepdims=True)
        pe = jnp.exp2(ext - m[HB:])
        ps = [jnp.exp2(tiles[t] - m) for t in range(nt)]
        p_main = jnp.concatenate(ps, axis=1).astype(bf16)
        lt = ps[0]
        for p in ps[1:]:
            lt = lt + p
        cm = _dot(p_main, vr[0:r0 + HB, :])
        lt = jnp.concatenate([lt[:HB], lt[HB:] + pe], axis=0)
        l = jnp.sum(lt, axis=1, keepdims=True)
        ce = _dot(pe.astype(bf16), vr[r0 + HB:r0 + BQ, :])
        cm = jnp.concatenate([cm[:HB], cm[HB:] + ce], axis=0)
        val = (cm * _recip(l)).astype(bf16)

        def store():
            big[rows(h * S + r0, BQ, BQ), :] = val
        return store

    def causal_tri():
        row = jax.lax.broadcasted_iota(jnp.int32, (HB, HB), 0)
        col = jax.lax.broadcasted_iota(jnp.int32, (HB, HB), 1)
        return col <= row

    def head_body(h, carry):
        hn = h + 1
        tri = causal_tri()
        va[0:2 * BQ, :] = vn[...]
        seq = [(h, i, va) for i in range(1, NQ)] + [(hn, 0, vn)]
        pend = []
        for hh, i, vr in seq:
            s_main, s_ext = qk(hh, i)
            if hh is hn:
                proj(hn, 1, True)
            elif i + 1 == NQ:
                proj(hn, 0, True)
            else:
                proj(h, i + 1, False)
            if hh is h and i == CONV_AT:
                gc = h // HG + 1
                convert_slice(jnp.minimum(gc, NG - 1), gc % 2, h % HG)
            if hh is h and i == EXT_AT:
                he = jnp.minimum(hn, H - 1)
                extract((he // HG) % 2, he % HG, hn % 2)
            while len(pend) >= LAG:
                pend.pop(0)()
            pend.append(softmax_pv(hh, i, s_main, s_ext, tri, vr))
        for st in pend:
            st()
        return carry

    def permute_rows(blk, slot, mc):
        for h4 in range(4):
            tb[slot, mc, pl.ds(h4, 32, stride=4), :] = blk[h4 * 32:(h4 + 1) * 32, :]

    def bprep_qkv(t, slot):
        part = t // 8
        g = t % 8
        for mc in range(M // 128):
            permute_rows(
                wqkv_s[mc * 128:(mc + 1) * 128, pl.ds(pl.multiple_of(t * 128, 128), 128)].astype(f32).T, slot, mc)
        for mc in range(M // 128):
            for i in range(8):
                wt_s[mc, rows(part * M + i * 128 + g * 16, 16, 16), :] = (
                    tb[slot, mc, i * 16:(i + 1) * 16, :].astype(bf16))

    def bprep_q_part(t, carry):
        for k in range(1, len(WQ_CHUNKS)):
            @pl.when(t == WQ_CHUNKS[k][0])
            def _():
                wait(cp_wq(k))
        bprep_qkv(t, 0)
        return carry

    def bprep_wo(g, slot):
        for nc in range(M // 128):
            permute_rows(wob_s[rows(g * 128, 128, 128), nc * 128:(nc + 1) * 128].astype(f32), slot, nc)
        for nc in range(M // 128):
            for i in range(8):
                wobp_s[nc, rows(i * 128 + g * 16, 16, 16), :] = tb[slot, nc, i * 16:(i + 1) * 16, :].astype(bf16)

    def b_proj(part, u):
        wt = jnp.concatenate([wt_s[mc, rows(part * M, M, M), :] for mc in range(8)], axis=1)
        res = _dot_nt(xb_s[rows(u * PR, PR, PR), :], wt)
        if not isinstance(part, int):
            res = res * jnp.where(part == 0, BDH ** -0.5 * LOG2E, 1.0)
        rr = rows(u * PR + HALO, PR, HALO)
        for j in range(8):
            qkv_s[part, j, rr, :] = res[:, j * 128:(j + 1) * 128]

    def b_proj_qk(it, carry):
        for k in range(2 * NPR):
            @pl.when(it == k)
            def _():
                wait(cp_set(k))
        b_proj(it // NPR, it % NPR)
        bprep_qkv(8 + 2 * it, 0)
        bprep_qkv(9 + 2 * it, 1)
        return carry

    def b_proj_v(u, carry):
        b_proj(2, u)
        for k in range(2):
            convert_slice(0, 0, 2 * u + k)
            bprep_wo(2 * u + k, k)
        return carry

    def b_attn_chunk(r0, cch, never, tok):
        a0 = cch * CH
        lane = jax.lax.broadcasted_iota(jnp.int32, (CH, 128), 1)
        b2 = (lane & 4) != 0
        b3 = (lane & 8) != 0
        qs = [qkv_s[0, j, pl.ds(r0 + (HALO + a0), CH), :] for j in range(8)]
        if tok is not None:
            qs = [jnp.where(never, tok, q) for q in qs]
        logit = []
        for w in range(BW):
            acc = None
            for j in range(8):
                term = qs[j] * qkv_s[1, j, pl.ds(r0 + (HALO + a0 - BDIL * w), CH), :]
                acc = term if acc is None else acc + term
            acc = acc + jnp.where(b2, pltpu.roll(acc, 4, 1), pltpu.roll(acc, 124, 1))
            acc = acc + jnp.where(b3, pltpu.roll(acc, 8, 1), pltpu.roll(acc, 120, 1))
            if a0 < BDIL * w:
                pos = jax.lax.broadcasted_iota(jnp.int32, (CH, 128), 0) + (r0 + a0)
                acc = jnp.where(pos >= BDIL * w, acc, NEG)
            logit.append(acc)
        mx = logit[0]
        for w in range(1, BW):
            mx = jnp.maximum(mx, logit[w])
        e = [jnp.exp2(lg - mx) for lg in logit]
        den = e[0]
        for w in range(1, BW):
            den = den + e[w]
        inv = _recip(den)
        e = [ew * inv for ew in e]
        outs = []
        for j in range(8):
            acc = None
            for w in range(BW):
                term = e[w] * qkv_s[2, j, pl.ds(r0 + (HALO + a0 - BDIL * w), CH), :]
                acc = term if acc is None else acc + term
            outs.append(acc)
        return outs

    @pl.when(step == 0)
    def _phase1():
        for k in range(len(WQ_CHUNKS)):
            start(cp_wq(k))
        for it in range(2 * NPR):
            start(cp_set(it))
        start(cp_mid())
        start(cp_late())
        zero_s[0] = 0
        for part in range(1, 3):
            qkv_s[part, :, 0:HALO, :] = jnp.zeros((8, HALO, 128), f32)
        wait(cp_wq(0))
        jax.lax.fori_loop(0, 8, bprep_q_part, 0)
        jax.lax.fori_loop(0, 2 * NPR, b_proj_qk, 0)
        wait(cp_mid())
        jax.lax.fori_loop(0, NPR, b_proj_v, 0)
        wait(cp_late())
        extract(0, 0, 0)
        proj(0, 0, True)
        s_main, s_ext = qk(0, 0)
        proj(0, 1, True)
        softmax_pv(0, 0, s_main, s_ext, causal_tri(), vn)()
        jax.lax.fori_loop(0, H, head_body, 0)

    @pl.when(step > 0)
    def _phase2():
        t = step - 1
        r0 = pl.multiple_of(t * BR, BR)
        never = zero_s[0] > 0
        ctx = jnp.concatenate([big[rows(h * S + r0, BR, BR), :] for h in range(H)], axis=1)
        nstage = (M // 128) * KS
        per = (BR // CH) // nstage
        kw = (H * D) // KS
        tok = None
        stage = 0
        half = []
        for p in range(M // 128):
            res = None
            for kk in range(KS):
                for cch in range(stage * per, (stage + 1) * per):
                    outs = b_attn_chunk(r0, cch, never, tok)
                    half.append(outs)
                    if len(half) * CH == 16:
                        a0 = (cch + 1) * CH - 16
                        for j in range(8):
                            ob_s[a0:a0 + 16, j * 128:(j + 1) * 128] = jnp.concatenate(
                                [hf[j] for hf in half], axis=0).astype(bf16)
                        half = []
                part = _dot(ctx[:, kk * kw:(kk + 1) * kw], wo_s[kk * kw:(kk + 1) * kw, p * 128:(p + 1) * 128])
                res = part if res is None else res + part
                tok = res[0:CH, :]
                stage += 1
            o_ref[:, p * 128:(p + 1) * 128] = res.astype(o_ref.dtype)
        wob = jnp.concatenate([wobp_s[nc] for nc in range(8)], axis=1)
        o_ref[:, M:2 * M] = _dot(ob_s[...], wob).astype(o_ref.dtype)


@jax.jit
def pallas_concat_heads__compressed_kv_cla__sliding_local_dilated__prompt_kernel(
    A_x: jax.Array,
    A_c_kv: jax.Array,
    A_w_q: jax.Array,
    A_w_uk: jax.Array,
    A_w_uv: jax.Array,
    A_w_o: jax.Array,
    B_x: jax.Array,
    B_wqkv: jax.Array,
    B_wo: jax.Array,
):
    x = A_x.reshape(S, M)
    c = A_c_kv.reshape(S, DC)
    wo = A_w_o.reshape(H * D, M)
    xb = B_x.reshape(S, M)

    any_spec = pl.BlockSpec(memory_space=pl.ANY)
    V = pltpu.VMEM
    scratch = [
        V((S, M), bf16),
        V((S, DC), bf16),
        V((NG, M, HG, D), bf16),
        V((NG, DC, HG, D), bf16),
        V((NG, DC, HG, D), bf16),
        V((2, M * 4, D), jnp.uint32),
        V((2, DC * 4, D), jnp.uint32),
        V((2, DC * 4, D), jnp.uint32),
        V((2, M + 2 * DC, D), bf16),
        V((S, D), bf16),
        V((S, D), bf16),
        V((2 * BQ, D), bf16),
        V(((H + 1) * S, D), bf16),
        V((H * D, M), bf16),
        V((S, M), bf16),
        V((M, 3 * M), bf16),
        V((M, M), bf16),
        V((8, 3 * M, 128), bf16),
        V((8, M, 128), bf16),
        V((2, 8, 128, 128), f32),
        V((3, 8, S + HALO, 128), f32),
        V((BR, M), bf16),
        pltpu.SMEM((1,), jnp.int32),
        pltpu.SemaphoreType.DMA((len(WQ_CHUNKS) + 2 * NPR + 2,)),
    ]
    out = pl.pallas_call(
        _kernel,
        grid=(1 + NB,),
        in_specs=[any_spec] * 9,
        out_specs=pl.BlockSpec((BR, 2 * M), lambda s: (jnp.maximum(s - 1, 0), 0)),
        out_shape=jax.ShapeDtypeStruct((S, 2 * M), bf16),
        scratch_shapes=scratch,
        compiler_params=pltpu.CompilerParams(
            dimension_semantics=("arbitrary",),
            vmem_limit_bytes=124 * 1024 * 1024,
            disable_bounds_checks=True,
        ),
        name="fused_mla_local",
    )(x, c, A_w_q, A_w_uk, A_w_uv, wo, xb, B_wqkv, B_wo)
    return out.reshape(1, S, 2 * M)
```

```python
import jax
import jax.numpy as jnp
import jax.experimental.pallas as pl
import jax.experimental.pallas.tpu as pltpu

bf16 = jnp.bfloat16
f32 = jnp.float32

S = 2048
H = 32
D = 128
M = 1024
DC = 512
HG = 8
NG = H // HG
BQ = 256
NQ = S // BQ
HB = 128
BW = 8
BDIL = 2
BH = 32
BDH = 32
HALO = 16
BR = 256
NB = S // BR
CH = 8
KS = 16
NPC = 2
LOG2E = 1.4426950408889634
NEG = -1e30
NT = (((1,), (1,)), ((), ()))
NWQ = 24
WQ_CHUNKS = ((0, 1), (1, 3), (4, 4))
PR = 512
NPR = S // PR
CONV_AT = 2
EXT_AT = 2
LAG = 2
KV_FIRST = False


def _dot(a, b):
    return jnp.dot(a, b, preferred_element_type=f32)


def _dot_nt(a, b):
    return jax.lax.dot_general(a, b, NT, preferred_element_type=f32)


def _recip(x):
    r = pl.reciprocal(x, approx=True)
    return r * (2.0 - x * r)


def _kernel(x_hbm, c_hbm, wq_hbm, wuk_hbm, wuv_hbm, wo_hbm, xb_hbm, wqkv_hbm, wob_hbm,
            o_ref,
            x_s, c_s, rawq, rawk, rawv, tq, tk, tv,
            wbuf, ka, va, vn, big, wo_s, xb_s, wqkv_s, wob_s, wt_s, wobp_s,
            tb, qkv_s, ob_s, zero_s, sems):
    step = pl.program_id(0)
    zz = step

    SEM_WQ, SEM_SET, SEM_LATE = 0, len(WQ_CHUNKS), len(WQ_CHUNKS) + 2 * NPR
    MQ, MK = M // HG, DC // HG

    def cp_slices(g, s0, n, sem):
        heads = pl.ds(g * HG, HG)
        return [
            pltpu.make_async_copy(wuk_hbm.at[pl.ds(s0 * MK, n * MK), heads, :], rawk.at[g, pl.ds(s0 * MK, n * MK)], sem),
            pltpu.make_async_copy(wuv_hbm.at[pl.ds(s0 * MK, n * MK), heads, :], rawv.at[g, pl.ds(s0 * MK, n * MK)], sem),
            pltpu.make_async_copy(wq_hbm.at[pl.ds(s0 * MQ, n * MQ), heads, :], rawq.at[g, pl.ds(s0 * MQ, n * MQ)], sem),
        ]

    def cp_wq(k):
        t0, nt = WQ_CHUNKS[k]
        cols = pl.ds(t0 * 128, nt * 128)
        return [pltpu.make_async_copy(wqkv_hbm.at[:, cols], wqkv_s.at[:, cols], sems.at[SEM_WQ + k])]

    def cp_set(it):
        sem = sems.at[SEM_SET + it]
        cols = pl.ds((8 + 2 * it) * 128, 256)
        cps = [pltpu.make_async_copy(wqkv_hbm.at[:, cols], wqkv_s.at[:, cols], sem)]
        if it < NPR:
            r = pl.ds(it * PR, PR)
            cps.insert(0, pltpu.make_async_copy(xb_hbm.at[r], xb_s.at[r], sem))
        return cps

    def cp_late():
        sem = sems.at[SEM_LATE]
        cps = [pltpu.make_async_copy(c_hbm, c_s, sem), pltpu.make_async_copy(x_hbm, x_s, sem)]
        for g in range(1, NG):
            cps += cp_slices(g, 0, HG, sem)
        return cps + [pltpu.make_async_copy(wo_hbm, wo_s, sem)]

    def cp_mid():
        sem = sems.at[SEM_LATE + 1]
        return cp_slices(0, 0, HG, sem) + [pltpu.make_async_copy(wob_hbm, wob_s, sem)]

    def start(cps):
        for cp in cps:
            cp.start()

    def wait(cps):
        for cp in cps:
            cp.wait()

    def rows(start, size, align):
        return pl.ds(start if isinstance(start, int) else pl.multiple_of(start, align), size)

    def convert_slice(g, par, sl):
        for raw, dst, n in ((rawq, tq, M // HG), (rawk, tk, DC // HG), (rawv, tv, DC // HG)):
            m0 = sl * n if isinstance(sl, int) else pl.multiple_of(sl * n, n)
            dst[par, pl.ds(m0 * 4, n * 4), :] = pltpu.bitcast(
                raw[g, pl.ds(m0, n)].reshape(n * HG, D), jnp.uint32)

    def extract(par, j, wp):
        shift = jnp.where(j % 2 == 0, 16, 0).astype(jnp.uint32)
        for src, r0, n in ((tq, 0, M), (tk, M, DC), (tv, M + DC, DC)):
            w = src[par, pl.ds(j // 2, n, stride=4), :]
            w = (w << shift) & jnp.uint32(0xFFFF0000)
            wbuf[wp, r0:r0 + n, :] = pltpu.bitcast(w, f32).astype(bf16)

    def proj(h, i, staged):
        r = slice(i * BQ, (i + 1) * BQ)
        wp = h % 2

        def q_part():
            q = _dot(x_s[r, :], wbuf[wp, 0:M, :])
            big[rows((h + zz) * S + i * BQ, BQ, BQ), :] = (q * (D ** -0.5 * LOG2E)).astype(bf16)

        def kv_part():
            wkv = jnp.concatenate([wbuf[wp, M:M + DC, :], wbuf[wp, M + DC:M + 2 * DC, :]], axis=1)
            kv = _dot(c_s[r, :], wkv)
            ka[r, :] = kv[:, :D].astype(bf16)
            if staged:
                vn[r, :] = kv[:, D:].astype(bf16)
            else:
                va[r, :] = kv[:, D:].astype(bf16)

        if KV_FIRST:
            kv_part()
            q_part()
        else:
            q_part()
            kv_part()

    def qk(h, i):
        r0 = i * BQ
        q = big[rows((h + zz) * S + r0, BQ, BQ), :]
        s_main = _dot_nt(q, ka[0:r0 + HB, :])
        q_lo = big[rows((h + zz) * S + r0 + HB, HB, HB), :]
        s_ext = _dot_nt(q_lo, ka[r0 + HB:r0 + BQ, :])
        return s_main, s_ext

    def softmax_pv(h, i, s_main, s_ext, tri, vr):
        r0 = i * BQ
        nt = 2 * i + 1
        tiles = [s_main[:, t * HB:(t + 1) * HB] for t in range(nt)]
        last = tiles[-1]
        tiles[-1] = jnp.concatenate([jnp.where(tri, last[:HB], NEG), last[HB:]], axis=0)
        ext = jnp.where(tri, s_ext, NEG)
        mt = tiles[0]
        for t in range(1, nt):
            mt = jnp.maximum(mt, tiles[t])
        mt = jnp.concatenate([mt[:HB], jnp.maximum(mt[HB:], ext)], axis=0)
        m = jnp.max(mt, axis=1, keepdims=True)
        pe = jnp.exp2(ext - m[HB:])
        ps = [jnp.exp2(tiles[t] - m) for t in range(nt)]
        p_main = jnp.concatenate(ps, axis=1).astype(bf16)
        lt = ps[0]
        for p in ps[1:]:
            lt = lt + p
        cm = _dot(p_main, vr[0:r0 + HB, :])
        lt = jnp.concatenate([lt[:HB], lt[HB:] + pe], axis=0)
        l = jnp.sum(lt, axis=1, keepdims=True)
        ce = _dot(pe.astype(bf16), vr[r0 + HB:r0 + BQ, :])
        cm = jnp.concatenate([cm[:HB], cm[HB:] + ce], axis=0)
        val = (cm * _recip(l)).astype(bf16)

        def store():
            big[rows(h * S + r0, BQ, BQ), :] = val
        return store

    def causal_tri():
        row = jax.lax.broadcasted_iota(jnp.int32, (HB, HB), 0)
        col = jax.lax.broadcasted_iota(jnp.int32, (HB, HB), 1)
        return col <= row

    def head_body(h, carry):
        hn = h + 1
        tri = causal_tri()
        va[0:2 * BQ, :] = vn[...]
        seq = [(h, i, va) for i in range(1, NQ)] + [(hn, 0, vn)]
        pend = []
        for hh, i, vr in seq:
            s_main, s_ext = qk(hh, i)
            if hh is hn:
                proj(hn, 1, True)
            elif i + 1 == NQ:
                proj(hn, 0, True)
            else:
                proj(h, i + 1, False)
            if hh is h and i == CONV_AT:
                gc = h // HG + 1
                convert_slice(jnp.minimum(gc, NG - 1), gc % 2, h % HG)
            if hh is h and i == EXT_AT:
                he = jnp.minimum(hn, H - 1)
                extract((he // HG) % 2, he % HG, hn % 2)
            while len(pend) >= LAG:
                pend.pop(0)()
            pend.append(softmax_pv(hh, i, s_main, s_ext, tri, vr))
        for st in pend:
            st()
        return carry

    def permute_rows(blk, slot, mc):
        for h4 in range(4):
            tb[slot, mc, pl.ds(h4, 32, stride=4), :] = blk[h4 * 32:(h4 + 1) * 32, :]

    def bprep_qkv(t, slot):
        part = t // 8
        g = t % 8
        for mc in range(M // 128):
            permute_rows(
                wqkv_s[mc * 128:(mc + 1) * 128, pl.ds(pl.multiple_of(t * 128, 128), 128)].astype(f32).T, slot, mc)
        for mc in range(M // 128):
            for i in range(8):
                wt_s[mc, rows(part * M + i * 128 + g * 16, 16, 16), :] = (
                    tb[slot, mc, i * 16:(i + 1) * 16, :].astype(bf16))

    def bprep_q_part(t, carry):
        for k in range(1, len(WQ_CHUNKS)):
            @pl.when(t == WQ_CHUNKS[k][0])
            def _():
                wait(cp_wq(k))
        bprep_qkv(t, 0)
        return carry

    def bprep_wo(g, slot):
        for nc in range(M // 128):
            permute_rows(wob_s[rows(g * 128, 128, 128), nc * 128:(nc + 1) * 128].astype(f32), slot, nc)
        for nc in range(M // 128):
            for i in range(8):
                wobp_s[nc, rows(i * 128 + g * 16, 16, 16), :] = tb[slot, nc, i * 16:(i + 1) * 16, :].astype(bf16)

    def b_proj(part, u):
        wt = jnp.concatenate([wt_s[mc, rows(part * M, M, M), :] for mc in range(8)], axis=1)
        res = _dot_nt(xb_s[rows(u * PR, PR, PR), :], wt)
        if not isinstance(part, int):
            res = res * jnp.where(part == 0, BDH ** -0.5 * LOG2E, 1.0)
        rr = rows(u * PR + HALO, PR, HALO)
        for j in range(8):
            qkv_s[part, j, rr, :] = res[:, j * 128:(j + 1) * 128]

    def b_proj_qk(it, carry):
        for k in range(2 * NPR):
            @pl.when(it == k)
            def _():
                wait(cp_set(k))
        b_proj(it // NPR, it % NPR)
        bprep_qkv(8 + 2 * it, 0)
        bprep_qkv(9 + 2 * it, 1)
        return carry

    def b_proj_v(u, carry):
        b_proj(2, u)
        for k in range(2):
            convert_slice(0, 0, 2 * u + k)
            bprep_wo(2 * u + k, k)
        return carry

    def b_attn_chunk(r0, cch, never, tok):
        a0 = cch * CH
        lane = jax.lax.broadcasted_iota(jnp.int32, (CH, 128), 1)
        b2 = (lane & 4) != 0
        b3 = (lane & 8) != 0
        qs = [qkv_s[0, j, pl.ds(r0 + (HALO + a0), CH), :] for j in range(8)]
        if tok is not None:
            qs = [jnp.where(never, tok, q) for q in qs]
        logit = []
        for w in range(BW):
            acc = None
            for j in range(8):
                term = qs[j] * qkv_s[1, j, pl.ds(r0 + (HALO + a0 - BDIL * w), CH), :]
                acc = term if acc is None else acc + term
            acc = acc + jnp.where(b2, pltpu.roll(acc, 4, 1), pltpu.roll(acc, 124, 1))
            acc = acc + jnp.where(b3, pltpu.roll(acc, 8, 1), pltpu.roll(acc, 120, 1))
            if a0 < BDIL * w:
                pos = jax.lax.broadcasted_iota(jnp.int32, (CH, 128), 0) + (r0 + a0)
                acc = jnp.where(pos >= BDIL * w, acc, NEG)
            logit.append(acc)
        mx = logit[0]
        for w in range(1, BW):
            mx = jnp.maximum(mx, logit[w])
        e = [jnp.exp2(lg - mx) for lg in logit]
        den = e[0]
        for w in range(1, BW):
            den = den + e[w]
        inv = _recip(den)
        e = [ew * inv for ew in e]
        outs = []
        for j in range(8):
            acc = None
            for w in range(BW):
                term = e[w] * qkv_s[2, j, pl.ds(r0 + (HALO + a0 - BDIL * w), CH), :]
                acc = term if acc is None else acc + term
            outs.append(acc)
        return outs

    @pl.when(step == 0)
    def _phase1():
        for k in range(len(WQ_CHUNKS)):
            start(cp_wq(k))
        for it in range(2 * NPR):
            start(cp_set(it))
        start(cp_mid())
        start(cp_late())
        zero_s[0] = 0
        for part in range(1, 3):
            qkv_s[part, :, 0:HALO, :] = jnp.zeros((8, HALO, 128), f32)
        wait(cp_wq(0))
        jax.lax.fori_loop(0, 8, bprep_q_part, 0)
        jax.lax.fori_loop(0, 2 * NPR, b_proj_qk, 0)
        wait(cp_mid())
        jax.lax.fori_loop(0, NPR, b_proj_v, 0)
        wait(cp_late())
        extract(0, 0, 0)
        proj(0, 0, True)
        s_main, s_ext = qk(0, 0)
        proj(0, 1, True)
        softmax_pv(0, 0, s_main, s_ext, causal_tri(), vn)()
        jax.lax.fori_loop(0, H, head_body, 0)

    @pl.when(step > 0)
    def _phase2():
        t = step - 1
        r0 = pl.multiple_of(t * BR, BR)
        never = zero_s[0] > 0
        ctx = jnp.concatenate([big[rows(h * S + r0, BR, BR), :] for h in range(H)], axis=1)
        nstage = NPC * KS
        per = (BR // CH) // nstage
        kw = (H * D) // KS
        nw = M // NPC
        tok = None
        stage = 0
        half = []
        for p in range(NPC):
            res = None
            for kk in range(KS):
                for cch in range(stage * per, (stage + 1) * per):
                    outs = b_attn_chunk(r0, cch, never, tok)
                    half.append(outs)
                    if len(half) * CH == 16:
                        a0 = (cch + 1) * CH - 16
                        for j in range(8):
                            ob_s[a0:a0 + 16, j * 128:(j + 1) * 128] = jnp.concatenate(
                                [hf[j] for hf in half], axis=0).astype(bf16)
                        half = []
                part = _dot(ctx[:, kk * kw:(kk + 1) * kw], wo_s[kk * kw:(kk + 1) * kw, p * nw:(p + 1) * nw])
                res = part if res is None else res + part
                tok = res[0:CH, 0:128]
                stage += 1
            o_ref[:, p * nw:(p + 1) * nw] = res.astype(o_ref.dtype)
        wob = jnp.concatenate([wobp_s[nc] for nc in range(8)], axis=1)
        o_ref[:, M:2 * M] = _dot(ob_s[...], wob).astype(o_ref.dtype)


@jax.jit
def pallas_concat_heads__compressed_kv_cla__sliding_local_dilated__prompt_kernel(
    A_x: jax.Array,
    A_c_kv: jax.Array,
    A_w_q: jax.Array,
    A_w_uk: jax.Array,
    A_w_uv: jax.Array,
    A_w_o: jax.Array,
    B_x: jax.Array,
    B_wqkv: jax.Array,
    B_wo: jax.Array,
):
    x = A_x.reshape(S, M)
    c = A_c_kv.reshape(S, DC)
    wo = A_w_o.reshape(H * D, M)
    xb = B_x.reshape(S, M)

    any_spec = pl.BlockSpec(memory_space=pl.ANY)
    V = pltpu.VMEM
    scratch = [
        V((S, M), bf16),
        V((S, DC), bf16),
        V((NG, M, HG, D), bf16),
        V((NG, DC, HG, D), bf16),
        V((NG, DC, HG, D), bf16),
        V((2, M * 4, D), jnp.uint32),
        V((2, DC * 4, D), jnp.uint32),
        V((2, DC * 4, D), jnp.uint32),
        V((2, M + 2 * DC, D), bf16),
        V((S, D), bf16),
        V((S, D), bf16),
        V((2 * BQ, D), bf16),
        V(((H + 1) * S, D), bf16),
        V((H * D, M), bf16),
        V((S, M), bf16),
        V((M, 3 * M), bf16),
        V((M, M), bf16),
        V((8, 3 * M, 128), bf16),
        V((8, M, 128), bf16),
        V((2, 8, 128, 128), f32),
        V((3, 8, S + HALO, 128), f32),
        V((BR, M), bf16),
        pltpu.SMEM((1,), jnp.int32),
        pltpu.SemaphoreType.DMA((len(WQ_CHUNKS) + 2 * NPR + 2,)),
    ]
    out = pl.pallas_call(
        _kernel,
        grid=(1 + NB,),
        in_specs=[any_spec] * 9,
        out_specs=pl.BlockSpec((BR, 2 * M), lambda s: (jnp.maximum(s - 1, 0), 0)),
        out_shape=jax.ShapeDtypeStruct((S, 2 * M), bf16),
        scratch_shapes=scratch,
        compiler_params=pltpu.CompilerParams(
            dimension_semantics=("arbitrary",),
            vmem_limit_bytes=124 * 1024 * 1024,
            disable_bounds_checks=True,
        ),
        name="fused_mla_local",
    )(x, c, A_w_q, A_w_uk, A_w_uv, wo, xb, B_wqkv, B_wo)
    return out.reshape(1, S, 2 * M)
```

```python
import jax
import jax.numpy as jnp
import jax.experimental.pallas as pl
import jax.experimental.pallas.tpu as pltpu

bf16 = jnp.bfloat16
f32 = jnp.float32

S = 2048
H = 32
D = 128
M = 1024
DC = 512
HG = 8
NG = H // HG
BQ = 256
NQ = S // BQ
HB = 128
BW = 8
BDIL = 2
BDH = 32
HALO = 16
BR = 256
NB = S // BR
CH = 8
KS = 16
NPC = 2
LOG2E = 1.4426950408889634
NEG = -1e30
NT = (((1,), (1,)), ((), ()))
NWQ = 24
WQ_CHUNKS = ((0, 1), (1, 3), (4, 4))
PR = 512
NPR = S // PR
CONV_AT = 2
EXT_AT = 2
LAG = 2


def _dot(a, b):
    return jnp.dot(a, b, preferred_element_type=f32)


def _dot_nt(a, b):
    return jax.lax.dot_general(a, b, NT, preferred_element_type=f32)


def _recip(x):
    r = pl.reciprocal(x, approx=True)
    return r * (2.0 - x * r)


def _kernel(x_hbm, c_hbm, wq_hbm, wuk_hbm, wuv_hbm, wo_hbm, xb_hbm, wqkv_hbm, wob_hbm,
            o_ref,
            x_s, c_s, rawq, rawk, rawv, tq, tk, tv,
            wbuf, ka, va, vn, big, wo_s, xb_s, wqkv_s, wob_s, wt_s, wobp_s,
            tb, qkv_s, ob_s, zero_s, sems):
    step = pl.program_id(0)
    zz = step

    SEM_WQ, SEM_SET, SEM_LATE = 0, len(WQ_CHUNKS), len(WQ_CHUNKS) + 2 * NPR
    MQ, MK = M // HG, DC // HG

    def cp_slices(g, s0, n, sem):
        heads = pl.ds(g * HG, HG)
        return [
            pltpu.make_async_copy(wuk_hbm.at[pl.ds(s0 * MK, n * MK), heads, :], rawk.at[g, pl.ds(s0 * MK, n * MK)], sem),
            pltpu.make_async_copy(wuv_hbm.at[pl.ds(s0 * MK, n * MK), heads, :], rawv.at[g, pl.ds(s0 * MK, n * MK)], sem),
            pltpu.make_async_copy(wq_hbm.at[pl.ds(s0 * MQ, n * MQ), heads, :], rawq.at[g, pl.ds(s0 * MQ, n * MQ)], sem),
        ]

    def cp_wq(k):
        t0, nt = WQ_CHUNKS[k]
        cols = pl.ds(t0 * 128, nt * 128)
        return [pltpu.make_async_copy(wqkv_hbm.at[:, cols], wqkv_s.at[:, cols], sems.at[SEM_WQ + k])]

    def cp_set(it):
        sem = sems.at[SEM_SET + it]
        cols = pl.ds((8 + 2 * it) * 128, 256)
        cps = [pltpu.make_async_copy(wqkv_hbm.at[:, cols], wqkv_s.at[:, cols], sem)]
        if it < NPR:
            r = pl.ds(it * PR, PR)
            cps.insert(0, pltpu.make_async_copy(xb_hbm.at[r], xb_s.at[r], sem))
        return cps

    def cp_late():
        sem = sems.at[SEM_LATE]
        cps = [pltpu.make_async_copy(c_hbm, c_s, sem), pltpu.make_async_copy(x_hbm, x_s, sem)]
        for g in range(1, NG):
            cps += cp_slices(g, 0, HG, sem)
        return cps + [pltpu.make_async_copy(wo_hbm, wo_s, sem)]

    def cp_mid():
        sem = sems.at[SEM_LATE + 1]
        return cp_slices(0, 0, HG, sem) + [pltpu.make_async_copy(wob_hbm, wob_s, sem)]

    def start(cps):
        for cp in cps:
            cp.start()

    def wait(cps):
        for cp in cps:
            cp.wait()

    def rows(start, size, align):
        return pl.ds(start if isinstance(start, int) else pl.multiple_of(start, align), size)

    def convert_slice(g, par, sl):
        for raw, dst, n in ((rawq, tq, M // HG), (rawk, tk, DC // HG), (rawv, tv, DC // HG)):
            m0 = sl * n if isinstance(sl, int) else pl.multiple_of(sl * n, n)
            dst[par, pl.ds(m0 * 4, n * 4), :] = pltpu.bitcast(
                raw[g, pl.ds(m0, n)].reshape(n * HG, D), jnp.uint32)

    def extract(par, j, wp):
        shift = jnp.where(j % 2 == 0, 16, 0).astype(jnp.uint32)
        for src, r0, n in ((tq, 0, M), (tk, M, DC), (tv, M + DC, DC)):
            w = src[par, pl.ds(j // 2, n, stride=4), :]
            w = (w << shift) & jnp.uint32(0xFFFF0000)
            wbuf[wp, r0:r0 + n, :] = pltpu.bitcast(w, f32).astype(bf16)

    def proj(h, i, staged):
        r = slice(i * BQ, (i + 1) * BQ)
        wp = h % 2
        q = _dot(x_s[r, :], wbuf[wp, 0:M, :])
        big[rows((h + zz) * S + i * BQ, BQ, BQ), :] = (q * (D ** -0.5 * LOG2E)).astype(bf16)
        wkv = jnp.concatenate([wbuf[wp, M:M + DC, :], wbuf[wp, M + DC:M + 2 * DC, :]], axis=1)
        kv = _dot(c_s[r, :], wkv)
        ka[r, :] = kv[:, :D].astype(bf16)
        if staged:
            vn[r, :] = kv[:, D:].astype(bf16)
        else:
            va[r, :] = kv[:, D:].astype(bf16)

    def qk(h, i):
        r0 = i * BQ
        q = big[rows((h + zz) * S + r0, BQ, BQ), :]
        s_main = _dot_nt(q, ka[0:r0 + HB, :])
        q_lo = big[rows((h + zz) * S + r0 + HB, HB, HB), :]
        s_ext = _dot_nt(q_lo, ka[r0 + HB:r0 + BQ, :])
        return s_main, s_ext

    def softmax_pv(h, i, s_main, s_ext, tri, vr):
        r0 = i * BQ
        nt = 2 * i + 1
        tiles = [s_main[:, t * HB:(t + 1) * HB] for t in range(nt)]
        last = tiles[-1]
        tiles[-1] = jnp.concatenate([jnp.where(tri, last[:HB], NEG), last[HB:]], axis=0)
        ext = jnp.where(tri, s_ext, NEG)
        mt = tiles[0]
        for t in range(1, nt):
            mt = jnp.maximum(mt, tiles[t])
        mt = jnp.concatenate([mt[:HB], jnp.maximum(mt[HB:], ext)], axis=0)
        m = jnp.max(mt, axis=1, keepdims=True)
        pe = jnp.exp2(ext - m[HB:])
        ps = [jnp.exp2(tiles[t] - m) for t in range(nt)]
        p_main = jnp.concatenate(ps, axis=1).astype(bf16)
        lt = ps[0]
        for p in ps[1:]:
            lt = lt + p
        cm = _dot(p_main, vr[0:r0 + HB, :])
        lt = jnp.concatenate([lt[:HB], lt[HB:] + pe], axis=0)
        l = jnp.sum(lt, axis=1, keepdims=True)
        ce = _dot(pe.astype(bf16), vr[r0 + HB:r0 + BQ, :])
        cm = jnp.concatenate([cm[:HB], cm[HB:] + ce], axis=0)
        val = (cm * _recip(l)).astype(bf16)

        def store():
            big[rows(h * S + r0, BQ, BQ), :] = val
        return store

    def causal_tri():
        row = jax.lax.broadcasted_iota(jnp.int32, (HB, HB), 0)
        col = jax.lax.broadcasted_iota(jnp.int32, (HB, HB), 1)
        return col <= row

    def head_body(h, carry):
        hn = h + 1
        tri = causal_tri()
        va[0:2 * BQ, :] = vn[...]
        seq = [(h, i, va) for i in range(1, NQ)] + [(hn, 0, vn)]
        pend = []
        for hh, i, vr in seq:
            s_main, s_ext = qk(hh, i)
            if hh is hn:
                proj(hn, 1, True)
            elif i + 1 == NQ:
                proj(hn, 0, True)
            else:
                proj(h, i + 1, False)
            if hh is h and i == CONV_AT:
                gc = h // HG + 1
                convert_slice(jnp.minimum(gc, NG - 1), gc % 2, h % HG)
            if hh is h and i == EXT_AT:
                he = jnp.minimum(hn, H - 1)
                extract((he // HG) % 2, he % HG, hn % 2)
            while len(pend) >= LAG:
                pend.pop(0)()
            pend.append(softmax_pv(hh, i, s_main, s_ext, tri, vr))
        for st in pend:
            st()
        return carry

    def permute_rows(blk, slot, mc):
        for h4 in range(4):
            tb[slot, mc, pl.ds(h4, 32, stride=4), :] = blk[h4 * 32:(h4 + 1) * 32, :]

    def bprep_qkv(t, slot):
        part = t // 8
        g = t % 8
        for mc in range(M // 128):
            permute_rows(
                wqkv_s[mc * 128:(mc + 1) * 128, pl.ds(pl.multiple_of(t * 128, 128), 128)].astype(f32).T, slot, mc)
        for mc in range(M // 128):
            for i in range(8):
                wt_s[mc, rows(part * M + i * 128 + g * 16, 16, 16), :] = (
                    tb[slot, mc, i * 16:(i + 1) * 16, :].astype(bf16))

    def bprep_q_part(t, carry):
        for k in range(1, len(WQ_CHUNKS)):
            @pl.when(t == WQ_CHUNKS[k][0])
            def _():
                wait(cp_wq(k))
        bprep_qkv(t, 0)
        return carry

    def bprep_wo(g, slot):
        for nc in range(M // 128):
            permute_rows(wob_s[rows(g * 128, 128, 128), nc * 128:(nc + 1) * 128].astype(f32), slot, nc)
        for nc in range(M // 128):
            for i in range(8):
                wobp_s[nc, rows(i * 128 + g * 16, 16, 16), :] = tb[slot, nc, i * 16:(i + 1) * 16, :].astype(bf16)

    def b_proj(part, u):
        wt = jnp.concatenate([wt_s[mc, rows(part * M, M, M), :] for mc in range(8)], axis=1)
        res = _dot_nt(xb_s[rows(u * PR, PR, PR), :], wt)
        if not isinstance(part, int):
            res = res * jnp.where(part == 0, BDH ** -0.5 * LOG2E, 1.0)
        rr = rows(u * PR + HALO, PR, HALO)
        for j in range(8):
            qkv_s[part, j, rr, :] = res[:, j * 128:(j + 1) * 128]

    def b_proj_qk(it, carry):
        for k in range(2 * NPR):
            @pl.when(it == k)
            def _():
                wait(cp_set(k))
        b_proj(it // NPR, it % NPR)
        bprep_qkv(8 + 2 * it, 0)
        bprep_qkv(9 + 2 * it, 1)
        return carry

    def b_proj_v(u, carry):
        b_proj(2, u)
        for k in range(2):
            convert_slice(0, 0, 2 * u + k)
            bprep_wo(2 * u + k, k)
        return carry

    def b_attn_chunk(r0, cch, never, tok):
        a0 = cch * CH
        lane = jax.lax.broadcasted_iota(jnp.int32, (CH, 128), 1)
        b2 = (lane & 4) != 0
        b3 = (lane & 8) != 0
        qs = [qkv_s[0, j, pl.ds(r0 + (HALO + a0), CH), :] for j in range(8)]
        if tok is not None:
            qs = [jnp.where(never, tok, q) for q in qs]
        logit = []
        for w in range(BW):
            acc = None
            for j in range(8):
                term = qs[j] * qkv_s[1, j, pl.ds(r0 + (HALO + a0 - BDIL * w), CH), :]
                acc = term if acc is None else acc + term
            acc = acc + jnp.where(b2, pltpu.roll(acc, 4, 1), pltpu.roll(acc, 124, 1))
            acc = acc + jnp.where(b3, pltpu.roll(acc, 8, 1), pltpu.roll(acc, 120, 1))
            if a0 < BDIL * w:
                pos = jax.lax.broadcasted_iota(jnp.int32, (CH, 128), 0) + (r0 + a0)
                acc = jnp.where(pos >= BDIL * w, acc, NEG)
            logit.append(acc)
        mx = logit[0]
        for w in range(1, BW):
            mx = jnp.maximum(mx, logit[w])
        e = [jnp.exp2(lg - mx) for lg in logit]
        den = e[0]
        for w in range(1, BW):
            den = den + e[w]
        inv = _recip(den)
        e = [ew * inv for ew in e]
        outs = []
        for j in range(8):
            acc = None
            for w in range(BW):
                term = e[w] * qkv_s[2, j, pl.ds(r0 + (HALO + a0 - BDIL * w), CH), :]
                acc = term if acc is None else acc + term
            outs.append(acc)
        return outs

    @pl.when(step == 0)
    def _phase1():
        for k in range(len(WQ_CHUNKS)):
            start(cp_wq(k))
        for it in range(2 * NPR):
            start(cp_set(it))
        start(cp_mid())
        start(cp_late())
        zero_s[0] = 0
        for part in range(1, 3):
            qkv_s[part, :, 0:HALO, :] = jnp.zeros((8, HALO, 128), f32)
        wait(cp_wq(0))
        jax.lax.fori_loop(0, 8, bprep_q_part, 0)
        jax.lax.fori_loop(0, 2 * NPR, b_proj_qk, 0)
        wait(cp_mid())
        jax.lax.fori_loop(0, NPR, b_proj_v, 0)
        wait(cp_late())
        extract(0, 0, 0)
        proj(0, 0, True)
        s_main, s_ext = qk(0, 0)
        proj(0, 1, True)
        softmax_pv(0, 0, s_main, s_ext, causal_tri(), vn)()
        jax.lax.fori_loop(0, H, head_body, 0)

    @pl.when(step > 0)
    def _phase2():
        t = step - 1
        r0 = pl.multiple_of(t * BR, BR)
        never = zero_s[0] > 0
        ctx = jnp.concatenate([big[rows(h * S + r0, BR, BR), :] for h in range(H)], axis=1)
        nstage = NPC * KS
        per = (BR // CH) // nstage
        kw = (H * D) // KS
        nw = M // NPC
        tok = None
        stage = 0
        half = []
        for p in range(NPC):
            res = None
            for kk in range(KS):
                for cch in range(stage * per, (stage + 1) * per):
                    outs = b_attn_chunk(r0, cch, never, tok)
                    half.append(outs)
                    if len(half) * CH == 16:
                        a0 = (cch + 1) * CH - 16
                        for j in range(8):
                            ob_s[a0:a0 + 16, j * 128:(j + 1) * 128] = jnp.concatenate(
                                [hf[j] for hf in half], axis=0).astype(bf16)
                        half = []
                part = _dot(ctx[:, kk * kw:(kk + 1) * kw], wo_s[kk * kw:(kk + 1) * kw, p * nw:(p + 1) * nw])
                res = part if res is None else res + part
                tok = res[0:CH, 0:128]
                stage += 1
            o_ref[:, p * nw:(p + 1) * nw] = res.astype(o_ref.dtype)
        wob = jnp.concatenate([wobp_s[nc] for nc in range(8)], axis=1)
        o_ref[:, M:2 * M] = _dot(ob_s[...], wob).astype(o_ref.dtype)


@jax.jit
def pallas_concat_heads__compressed_kv_cla__sliding_local_dilated__prompt_kernel(
    A_x: jax.Array,
    A_c_kv: jax.Array,
    A_w_q: jax.Array,
    A_w_uk: jax.Array,
    A_w_uv: jax.Array,
    A_w_o: jax.Array,
    B_x: jax.Array,
    B_wqkv: jax.Array,
    B_wo: jax.Array,
):
    x = A_x.reshape(S, M)
    c = A_c_kv.reshape(S, DC)
    wo = A_w_o.reshape(H * D, M)
    xb = B_x.reshape(S, M)

    any_spec = pl.BlockSpec(memory_space=pl.ANY)
    V = pltpu.VMEM
    scratch = [
        V((S, M), bf16),
        V((S, DC), bf16),
        V((NG, M, HG, D), bf16),
        V((NG, DC, HG, D), bf16),
        V((NG, DC, HG, D), bf16),
        V((2, M * 4, D), jnp.uint32),
        V((2, DC * 4, D), jnp.uint32),
        V((2, DC * 4, D), jnp.uint32),
        V((2, M + 2 * DC, D), bf16),
        V((S, D), bf16),
        V((S, D), bf16),
        V((2 * BQ, D), bf16),
        V(((H + 1) * S, D), bf16),
        V((H * D, M), bf16),
        V((S, M), bf16),
        V((M, 3 * M), bf16),
        V((M, M), bf16),
        V((8, 3 * M, 128), bf16),
        V((8, M, 128), bf16),
        V((2, 8, 128, 128), f32),
        V((3, 8, S + HALO, 128), f32),
        V((BR, M), bf16),
        pltpu.SMEM((1,), jnp.int32),
        pltpu.SemaphoreType.DMA((len(WQ_CHUNKS) + 2 * NPR + 2,)),
    ]
    out = pl.pallas_call(
        _kernel,
        grid=(1 + NB,),
        in_specs=[any_spec] * 9,
        out_specs=pl.BlockSpec((BR, 2 * M), lambda s: (jnp.maximum(s - 1, 0), 0)),
        out_shape=jax.ShapeDtypeStruct((S, 2 * M), bf16),
        scratch_shapes=scratch,
        compiler_params=pltpu.CompilerParams(
            dimension_semantics=("arbitrary",),
            vmem_limit_bytes=124 * 1024 * 1024,
        ),
        name="fused_mla_local",
    )(x, c, A_w_q, A_w_uk, A_w_uv, wo, xb, B_wqkv, B_wo)
    return out.reshape(1, S, 2 * M)
```

```python
import jax
import jax.numpy as jnp
import jax.experimental.pallas as pl
import jax.experimental.pallas.tpu as pltpu

bf16 = jnp.bfloat16
f32 = jnp.float32

S = 2048
H = 32
D = 128
M = 1024
DC = 512
HG = 8
NG = H // HG
BQ = 256
NQ = S // BQ
HB = 128
BW = 8
BDIL = 2
BDH = 32
HALO = 16
BR = 256
NB = S // BR
CH = 8
KS = 16
NPC = 2
LOG2E = 1.4426950408889634
NEG = -1e30
NT = (((1,), (1,)), ((), ()))
NWQ = 24
WQ_CHUNKS = ((0, 1), (1, 3), (4, 4))
PR = 512
NPR = S // PR
CONV_AT = 2
EXT_AT = 2
LAG = 2


def _dot(a, b):
    return jnp.dot(a, b, preferred_element_type=f32)


def _dot_nt(a, b):
    return jax.lax.dot_general(a, b, NT, preferred_element_type=f32)


def _recip(x):
    r = pl.reciprocal(x, approx=True)
    return r * (2.0 - x * r)


def _kernel(x_hbm, c_hbm, wq_hbm, wuk_hbm, wuv_hbm, wo_hbm, xb_hbm, wqkv_hbm, wob_hbm,
            o_ref,
            x_s, c_s, rawq, rawk, rawv, tq, tk, tv,
            wbuf, ka, va, vn, big, wo_s, xb_s, wqkv_s, wob_s, wt_s, wobp_s,
            tb, qkv_s, ob_s, zero_s, sems):
    step = pl.program_id(0)
    zz = step

    SEM_WQ, SEM_SET, SEM_LATE = 0, len(WQ_CHUNKS), len(WQ_CHUNKS) + 2 * NPR
    MQ, MK = M // HG, DC // HG

    def cp_slices(g, s0, n, sem):
        heads = pl.ds(g * HG, HG)
        return [
            pltpu.make_async_copy(wuk_hbm.at[pl.ds(s0 * MK, n * MK), heads, :], rawk.at[g, pl.ds(s0 * MK, n * MK)], sem),
            pltpu.make_async_copy(wuv_hbm.at[pl.ds(s0 * MK, n * MK), heads, :], rawv.at[g, pl.ds(s0 * MK, n * MK)], sem),
            pltpu.make_async_copy(wq_hbm.at[pl.ds(s0 * MQ, n * MQ), heads, :], rawq.at[g, pl.ds(s0 * MQ, n * MQ)], sem),
        ]

    def cp_wq(k):
        t0, nt = WQ_CHUNKS[k]
        cols = pl.ds(t0 * 128, nt * 128)
        return [pltpu.make_async_copy(wqkv_hbm.at[:, cols], wqkv_s.at[:, cols], sems.at[SEM_WQ + k])]

    def cp_set(it):
        sem = sems.at[SEM_SET + it]
        cols = pl.ds((8 + 2 * it) * 128, 256)
        cps = [pltpu.make_async_copy(wqkv_hbm.at[:, cols], wqkv_s.at[:, cols], sem)]
        if it < NPR:
            r = pl.ds(it * PR, PR)
            cps.insert(0, pltpu.make_async_copy(xb_hbm.at[r], xb_s.at[r], sem))
        return cps

    def cp_late():
        sem = sems.at[SEM_LATE]
        cps = [pltpu.make_async_copy(c_hbm, c_s, sem), pltpu.make_async_copy(x_hbm, x_s, sem)]
        for g in range(1, NG):
            cps += cp_slices(g, 0, HG, sem)
        return cps + [pltpu.make_async_copy(wo_hbm, wo_s, sem)]

    def cp_mid():
        sem = sems.at[SEM_LATE + 1]
        return cp_slices(0, 0, HG, sem) + [pltpu.make_async_copy(wob_hbm, wob_s, sem)]

    def start(cps):
        for cp in cps:
            cp.start()

    def wait(cps):
        for cp in cps:
            cp.wait()

    def rows(start, size, align):
        return pl.ds(start if isinstance(start, int) else pl.multiple_of(start, align), size)

    def convert_slice(g, par, sl):
        for raw, dst, n in ((rawq, tq, M // HG), (rawk, tk, DC // HG), (rawv, tv, DC // HG)):
            m0 = sl * n if isinstance(sl, int) else pl.multiple_of(sl * n, n)
            dst[par, pl.ds(m0 * 4, n * 4), :] = pltpu.bitcast(
                raw[g, pl.ds(m0, n)].reshape(n * HG, D), jnp.uint32)

    def extract(par, j, wp):
        shift = jnp.where(j % 2 == 0, 16, 0).astype(jnp.uint32)
        for src, r0, n in ((tq, 0, M), (tk, M, DC), (tv, M + DC, DC)):
            w = src[par, pl.ds(j // 2, n, stride=4), :]
            w = (w << shift) & jnp.uint32(0xFFFF0000)
            wbuf[wp, r0:r0 + n, :] = pltpu.bitcast(w, f32).astype(bf16)

    def proj(h, i, staged):
        r = slice(i * BQ, (i + 1) * BQ)
        wp = h % 2
        q = _dot(x_s[r, :], wbuf[wp, 0:M, :])
        big[rows((h + zz) * S + i * BQ, BQ, BQ), :] = (q * (D ** -0.5 * LOG2E)).astype(bf16)
        wkv = jnp.concatenate([wbuf[wp, M:M + DC, :], wbuf[wp, M + DC:M + 2 * DC, :]], axis=1)
        kv = _dot(c_s[r, :], wkv)
        ka[r, :] = kv[:, :D].astype(bf16)
        if staged:
            vn[r, :] = kv[:, D:].astype(bf16)
        else:
            va[r, :] = kv[:, D:].astype(bf16)

    def qk(h, i):
        r0 = i * BQ
        q = big[rows((h + zz) * S + r0, BQ, BQ), :]
        s_main = _dot_nt(q, ka[0:r0 + HB, :])
        q_lo = big[rows((h + zz) * S + r0 + HB, HB, HB), :]
        s_ext = _dot_nt(q_lo, ka[r0 + HB:r0 + BQ, :])
        return s_main, s_ext

    def softmax_pv(h, i, s_main, s_ext, tri, vr):
        r0 = i * BQ
        nt = 2 * i + 1
        tiles = [s_main[:, t * HB:(t + 1) * HB] for t in range(nt)]
        last = tiles[-1]
        tiles[-1] = jnp.concatenate([jnp.where(tri, last[:HB], NEG), last[HB:]], axis=0)
        ext = jnp.where(tri, s_ext, NEG)
        mt = tiles[0]
        for t in range(1, nt):
            mt = jnp.maximum(mt, tiles[t])
        mt = jnp.concatenate([mt[:HB], jnp.maximum(mt[HB:], ext)], axis=0)
        m = jnp.max(mt, axis=1, keepdims=True)
        pe = jnp.exp2(ext - m[HB:])
        ps = [jnp.exp2(tiles[t] - m) for t in range(nt)]
        p_main = jnp.concatenate(ps, axis=1).astype(bf16)
        lt = ps[0]
        for p in ps[1:]:
            lt = lt + p
        cm = _dot(p_main, vr[0:r0 + HB, :])
        lt = jnp.concatenate([lt[:HB], lt[HB:] + pe], axis=0)
        l = jnp.sum(lt, axis=1, keepdims=True)
        ce = _dot(pe.astype(bf16), vr[r0 + HB:r0 + BQ, :])
        cm = jnp.concatenate([cm[:HB], cm[HB:] + ce], axis=0)
        val = (cm * _recip(l)).astype(bf16)

        def store():
            big[rows(h * S + r0, BQ, BQ), :] = val
        return store

    def causal_tri():
        row = jax.lax.broadcasted_iota(jnp.int32, (HB, HB), 0)
        col = jax.lax.broadcasted_iota(jnp.int32, (HB, HB), 1)
        return col <= row

    def head_body(h, carry):
        hn = h + 1
        tri = causal_tri()
        va[0:2 * BQ, :] = vn[...]
        seq = [(h, i, va) for i in range(1, NQ)] + [(hn, 0, vn)]
        pend = []
        for hh, i, vr in seq:
            s_main, s_ext = qk(hh, i)
            if hh is hn:
                proj(hn, 1, True)
            elif i + 1 == NQ:
                proj(hn, 0, True)
            else:
                proj(h, i + 1, False)
            if hh is h and i == CONV_AT:
                gc = h // HG + 1
                convert_slice(jnp.minimum(gc, NG - 1), gc % 2, h % HG)
            if hh is h and i == EXT_AT:
                he = jnp.minimum(hn, H - 1)
                extract((he // HG) % 2, he % HG, hn % 2)
            while len(pend) >= LAG:
                pend.pop(0)()
            pend.append(softmax_pv(hh, i, s_main, s_ext, tri, vr))
        for st in pend:
            st()
        return carry

    def permute_rows(blk, slot, mc):
        for h4 in range(4):
            tb[slot, mc, pl.ds(h4, 32, stride=4), :] = blk[h4 * 32:(h4 + 1) * 32, :]

    def bprep_qkv(t, slot):
        part = t // 8
        g = t % 8
        for mc in range(M // 128):
            permute_rows(
                wqkv_s[mc * 128:(mc + 1) * 128, pl.ds(pl.multiple_of(t * 128, 128), 128)].astype(f32).T, slot, mc)
        for mc in range(M // 128):
            for i in range(8):
                wt_s[mc, rows(part * M + i * 128 + g * 16, 16, 16), :] = (
                    tb[slot, mc, i * 16:(i + 1) * 16, :].astype(bf16))

    def bprep_q_part(t, carry):
        for k in range(1, len(WQ_CHUNKS)):
            @pl.when(t == WQ_CHUNKS[k][0])
            def _():
                wait(cp_wq(k))
        bprep_qkv(t, 0)
        return carry

    def bprep_wo(g, slot):
        for nc in range(M // 128):
            permute_rows(wob_s[rows(g * 128, 128, 128), nc * 128:(nc + 1) * 128].astype(f32), slot, nc)
        for nc in range(M // 128):
            for i in range(8):
                wobp_s[nc, rows(i * 128 + g * 16, 16, 16), :] = tb[slot, nc, i * 16:(i + 1) * 16, :].astype(bf16)

    def b_proj(part, u):
        wt = jnp.concatenate([wt_s[mc, rows(part * M, M, M), :] for mc in range(8)], axis=1)
        res = _dot_nt(xb_s[rows(u * PR, PR, PR), :], wt)
        if not isinstance(part, int):
            res = res * jnp.where(part == 0, BDH ** -0.5 * LOG2E, 1.0)
        rr = rows(u * PR + HALO, PR, HALO)
        for j in range(8):
            qkv_s[part, j, rr, :] = res[:, j * 128:(j + 1) * 128]

    def b_proj_qk(it, carry):
        for k in range(2 * NPR):
            @pl.when(it == k)
            def _():
                wait(cp_set(k))
        b_proj(it // NPR, it % NPR)
        bprep_qkv(8 + 2 * it, 0)
        bprep_qkv(9 + 2 * it, 1)
        return carry

    def b_proj_v(u, carry):
        b_proj(2, u)
        for k in range(2):
            convert_slice(0, 0, 2 * u + k)
            bprep_wo(2 * u + k, k)
        return carry

    def b_attn_chunk(r0, cch, never, tok):
        a0 = cch * CH
        lane = jax.lax.broadcasted_iota(jnp.int32, (CH, 128), 1)
        b2 = (lane & 4) != 0
        b3 = (lane & 8) != 0
        qs = [qkv_s[0, j, pl.ds(r0 + (HALO + a0), CH), :] for j in range(8)]
        if tok is not None:
            qs = [jnp.where(never, tok, q) for q in qs]
        logit = []
        for w in range(BW):
            acc = None
            for j in range(8):
                term = qs[j] * qkv_s[1, j, pl.ds(r0 + (HALO + a0 - BDIL * w), CH), :]
                acc = term if acc is None else acc + term
            acc = acc + jnp.where(b2, pltpu.roll(acc, 4, 1), pltpu.roll(acc, 124, 1))
            acc = acc + jnp.where(b3, pltpu.roll(acc, 8, 1), pltpu.roll(acc, 120, 1))
            if a0 < BDIL * w:
                pos = jax.lax.broadcasted_iota(jnp.int32, (CH, 128), 0) + (r0 + a0)
                acc = jnp.where(pos >= BDIL * w, acc, NEG)
            logit.append(acc)
        mx = logit[0]
        for w in range(1, BW):
            mx = jnp.maximum(mx, logit[w])
        e = [jnp.exp2(lg - mx) for lg in logit]
        den = e[0]
        for w in range(1, BW):
            den = den + e[w]
        inv = _recip(den)
        e = [ew * inv for ew in e]
        outs = []
        for j in range(8):
            acc = None
            for w in range(BW):
                term = e[w] * qkv_s[2, j, pl.ds(r0 + (HALO + a0 - BDIL * w), CH), :]
                acc = term if acc is None else acc + term
            outs.append(acc)
        return outs

    @pl.when(step == 0)
    def _phase1():
        for k in range(len(WQ_CHUNKS)):
            start(cp_wq(k))
        for it in range(2 * NPR):
            start(cp_set(it))
        start(cp_mid())
        start(cp_late())
        zero_s[0] = 0
        for part in range(1, 3):
            qkv_s[part, :, 0:HALO, :] = jnp.zeros((8, HALO, 128), f32)
        wait(cp_wq(0))
        jax.lax.fori_loop(0, 8, bprep_q_part, 0)
        jax.lax.fori_loop(0, 2 * NPR, b_proj_qk, 0)
        wait(cp_mid())
        jax.lax.fori_loop(0, NPR, b_proj_v, 0)
        wait(cp_late())
        extract(0, 0, 0)
        proj(0, 0, True)
        s_main, s_ext = qk(0, 0)
        proj(0, 1, True)
        softmax_pv(0, 0, s_main, s_ext, causal_tri(), vn)()
        jax.lax.fori_loop(0, H, head_body, 0)

    @pl.when(step > 0)
    def _phase2():
        t = step - 1
        r0 = pl.multiple_of(t * BR, BR)
        never = zero_s[0] > 0
        ctx = jnp.concatenate([big[rows(h * S + r0, BR, BR), :] for h in range(H)], axis=1)
        nstage = NPC * KS
        kw = (H * D) // KS
        nw = M // NPC
        stage = 0
        half = []
        for p in range(NPC):
            res = None
            for kk in range(KS):
                part = _dot(ctx[:, kk * kw:(kk + 1) * kw], wo_s[kk * kw:(kk + 1) * kw, p * nw:(p + 1) * nw])
                res = part if res is None else res + part
                tok = res[0:CH, 0:128]
                if stage < nstage - 2:
                    todo = [stage]
                elif stage == nstage - 2:
                    todo = [stage, stage + 1]
                else:
                    todo = []
                for cch in todo:
                    outs = b_attn_chunk(r0, cch, never, tok)
                    half.append(outs)
                    if len(half) * CH == 16:
                        a0 = (cch + 1) * CH - 16
                        for j in range(8):
                            ob_s[a0:a0 + 16, j * 128:(j + 1) * 128] = jnp.concatenate(
                                [hf[j] for hf in half], axis=0).astype(bf16)
                        half = []
                stage += 1
            o_ref[:, p * nw:(p + 1) * nw] = res.astype(o_ref.dtype)
        wob = jnp.concatenate([wobp_s[nc] for nc in range(8)], axis=1)
        o_ref[:, M:2 * M] = _dot(ob_s[...], wob).astype(o_ref.dtype)


@jax.jit
def pallas_concat_heads__compressed_kv_cla__sliding_local_dilated__prompt_kernel(
    A_x: jax.Array,
    A_c_kv: jax.Array,
    A_w_q: jax.Array,
    A_w_uk: jax.Array,
    A_w_uv: jax.Array,
    A_w_o: jax.Array,
    B_x: jax.Array,
    B_wqkv: jax.Array,
    B_wo: jax.Array,
):
    x = A_x.reshape(S, M)
    c = A_c_kv.reshape(S, DC)
    wo = A_w_o.reshape(H * D, M)
    xb = B_x.reshape(S, M)

    any_spec = pl.BlockSpec(memory_space=pl.ANY)
    V = pltpu.VMEM
    scratch = [
        V((S, M), bf16),
        V((S, DC), bf16),
        V((NG, M, HG, D), bf16),
        V((NG, DC, HG, D), bf16),
        V((NG, DC, HG, D), bf16),
        V((2, M * 4, D), jnp.uint32),
        V((2, DC * 4, D), jnp.uint32),
        V((2, DC * 4, D), jnp.uint32),
        V((2, M + 2 * DC, D), bf16),
        V((S, D), bf16),
        V((S, D), bf16),
        V((2 * BQ, D), bf16),
        V(((H + 1) * S, D), bf16),
        V((H * D, M), bf16),
        V((S, M), bf16),
        V((M, 3 * M), bf16),
        V((M, M), bf16),
        V((8, 3 * M, 128), bf16),
        V((8, M, 128), bf16),
        V((2, 8, 128, 128), f32),
        V((3, 8, S + HALO, 128), f32),
        V((BR, M), bf16),
        pltpu.SMEM((1,), jnp.int32),
        pltpu.SemaphoreType.DMA((len(WQ_CHUNKS) + 2 * NPR + 2,)),
    ]
    out = pl.pallas_call(
        _kernel,
        grid=(1 + NB,),
        in_specs=[any_spec] * 9,
        out_specs=pl.BlockSpec((BR, 2 * M), lambda s: (jnp.maximum(s - 1, 0), 0)),
        out_shape=jax.ShapeDtypeStruct((S, 2 * M), bf16),
        scratch_shapes=scratch,
        compiler_params=pltpu.CompilerParams(
            dimension_semantics=("arbitrary",),
            vmem_limit_bytes=124 * 1024 * 1024,
        ),
        name="fused_mla_local",
    )(x, c, A_w_q, A_w_uk, A_w_uv, wo, xb, B_wqkv, B_wo)
    return out.reshape(1, S, 2 * M)
```
